```python
import os as _os
_os.environ.setdefault('JAX_PLATFORMS', 'cpu')
import jax
import jax.numpy as jnp

def _softmax(x, axis=-1):
    return jax.nn.softmax(x, axis=axis)

def _gelu(x):
    return jax.nn.gelu(x, approximate=True)

def _silu(x):
    return jax.nn.silu(x)

def _sigmoid(x):
    return jax.nn.sigmoid(x)

def _layernorm(x, axis=-1, eps=1e-05):
    m = jnp.mean(x, axis=axis, keepdims=True)
    v = jnp.var(x, axis=axis, keepdims=True)
    return (x - m) / jnp.sqrt(v + eps)

def _scatter_add(tgt, idx, src, axis=0):
    return tgt.at[idx].add(src)

def _segment_sum(src, seg, n):
    return jax.ops.segment_sum(src, seg, n)

class _Rng:

    def __init__(self, key):
        self._k = key

    def _next(self):
        self._k, sub = jax.random.split(self._k)
        return sub

    def normal(self, shape):
        return jax.random.normal(self._next(), shape, dtype=jnp.bfloat16)

    def randint(self, lo, hi, shape):
        return jax.random.randint(self._next(), shape, lo, hi, dtype=jnp.int32)

    def uniform(self, shape, lo=0.0, hi=1.0):
        return jax.random.uniform(self._next(), shape, jnp.bfloat16, lo, hi)

    def permutation(self, n):
        return jax.random.permutation(self._next(), n)
kernel_name = 'recurrent_scan__memory_aug_recurrent_mem_tr__mixer_gmlp__prompt'

def setup_inputs():
    _rng = _Rng(jax.random.key(int.from_bytes(__import__("os").urandom(4), "little")))
    _w = lambda a: (lambda t: t.astype(jnp.bfloat16) if jnp.issubdtype(t.dtype, jnp.floating) else t)(jnp.asarray(a))

    def _A_setup():
        B, S, Dm = (1, 2048, 640)
        H, Dh = (32, 128)
        M, seg = (8, 32)
        seg = min(seg, S)
        S = S // seg * seg
        return {'x': _w((lambda *s: _rng.normal(s) * 0.05)(B, S, Dm)), 'mem0': _w((lambda *s: _rng.normal(s) * 0.1)(B, M, Dm)), 'Wq': _w((lambda *s: _rng.normal(s) * 1.6)(Dm, H, Dh) * Dm ** (-0.5)), 'Wk': _w((lambda *s: _rng.normal(s) * 1.6)(Dm, H, Dh) * Dm ** (-0.5)), 'Wv': _w((lambda *s: _rng.normal(s) * 0.1)(Dm, H, Dh) * Dm ** (-0.5)), 'Wo': _w((lambda *s: _rng.normal(s) * 0.1)(H, Dh, Dm) * (H * Dh) ** (-0.5)), 'seg_len': seg}
    _A_in = _A_setup()

    def _B_setup():
        B, S, D, F = (1, 2048, 640, 1728)
        Fh = F // 2
        return {'x': _w((lambda *s: _rng.normal(s) * 0.05)(B, S, D)), 'w_in': _w((lambda *s: _rng.normal(s) * 0.8)(D, 2 * Fh)), 'w_sp': _w(0.01 * (lambda *s: _rng.normal(s) * 0.8)(S, S)), 'b_sp': _w(1.0 + 0.01 * (lambda *s: _rng.normal(s) * 0.05)(S)), 'w_out': _w((lambda *s: _rng.normal(s) * 0.05)(Fh, D))}
    _B_in = _B_setup()
    return {'A_x': _A_in['x'], 'A_mem0': _A_in['mem0'], 'A_Wq': _A_in['Wq'], 'A_Wk': _A_in['Wk'], 'A_Wv': _A_in['Wv'], 'A_Wo': _A_in['Wo'], 'A_seg_len': _A_in['seg_len'], 'B_x': _B_in['x'], 'B_w_in': _B_in['w_in'], 'B_w_sp': _B_in['w_sp'], 'B_b_sp': _B_in['b_sp'], 'B_w_out': _B_in['w_out']}

def reference(A_x, A_mem0, A_Wq, A_Wk, A_Wv, A_Wo, A_seg_len, B_x, B_w_in, B_w_sp, B_b_sp, B_w_out):

    def _A_ref(x, mem0, Wq, Wk, Wv, Wo, seg_len):
        B, S, Dm = x.shape
        H, Dh = (Wq.shape[1], Wq.shape[2])
        M = mem0.shape[1]
        scale = Dh ** (-0.5)
        n_seg = S // seg_len
        L = M + seg_len
        idx = jnp.arange(L)
        mask = (idx[:, None] < M) | (idx[:, None] >= idx[None, :])
        mem = mem0
        outs = []
        for s in range(n_seg):
            xs = x[:, s * seg_len:(s + 1) * seg_len, :].copy()
            h = jnp.concatenate([mem, xs], axis=1)
            q = jnp.einsum('btd,dhe->bhte', h, Wq)
            k = jnp.einsum('btd,dhe->bhte', h, Wk)
            v = jnp.einsum('btd,dhe->bhte', h, Wv)
            scores = jnp.einsum('bhqe,bhke->bhqk', q, k) * scale
            scores = jnp.where(mask[None, None], scores, -1000000000.0)
            p = _softmax(scores, axis=-1)
            o = jnp.einsum('bhqk,bhke->bhqe', p, v)
            o = jnp.einsum('bhte,hed->btd', o, Wo)
            mem = o[:, :M, :].copy()
            outs.append(o[:, M:, :])
        return jnp.concatenate(outs, axis=1)

    def _B_ref(x, w_in, w_sp, b_sp, w_out):
        B, S, D = x.shape
        F = w_in.shape[-1]
        Fh = F // 2
        z = _gelu(jnp.einsum('bsd,df->bsf', x, w_in))
        z1 = z[..., :Fh].copy()
        z2 = _layernorm(z[..., Fh:], axis=-1)
        g = jnp.einsum('ts,bsf->btf', w_sp, z2) + b_sp[None, :, None]
        return jnp.einsum('bsf,fd->bsd', z1 * g, w_out)
    x = A_x
    xn = _layernorm(x, axis=-1)
    s = _A_ref(xn, A_mem0, A_Wq, A_Wk, A_Wv, A_Wo, A_seg_len)
    g = _silu(_B_ref(xn, B_w_in, B_w_sp, B_b_sp, B_w_out))
    return x + s * g
```

```python
import functools
import jax
import jax.numpy as jnp
from jax import lax
import jax.experimental.pallas as pl
import jax.experimental.pallas.tpu as pltpu

F32 = jnp.float32
BF16 = jnp.bfloat16
U32 = jnp.uint32

S, D, H, DH, M, SEG = 2048, 640, 32, 128, 8, 32
FH = 864
NPAIR = S // (2 * SEG)
EPS = 1e-5
RB = 256
NB1 = S // RB
R0 = 512
RB2 = 128
NB2 = R0 // RB2
GR = (S - R0) // NPAIR
NF = 7
WC = 128
NWC = D // WC
WSP_A = 6
SK_S = 2
SK_PV = 5
SCHED = 'A32:w0,A33:w0,A34:w0,A35:w0,A36:w0,A99:g1,B4:g2,B9:g3,B14:g4,B19:g5,B24:g6,B32:m0m1,B33:m2m3,B34:m4w0,B35:w0,B36:w1,B99:n0'

SEM_X = 0
SEM_WIN = 3
SEM_W = 4
SEM_WOUT = 8
SEM_WSP = 9
SEM_WO = 15
NSEM = 16
NJ = 3 * H // 2
JPI = NJ // NB2


def _bf(x):
    return pltpu.bitcast(x, BF16)


def _u32(x):
    return pltpu.bitcast(x, U32)


def _dot(a, b):
    return jnp.dot(a, b, preferred_element_type=F32)


def _dot_nt(a, b):
    return lax.dot_general(a, b, (((1,), (1,)), ((), ())), preferred_element_type=F32)


def _gelu(x):
    c = 0.7978845608028654
    return 0.5 * x * (1.0 + jnp.tanh(c * (x + 0.044715 * (x * x * x))))


def _masks():
    qi = lax.broadcasted_iota(jnp.int32, (32, 48), 0)
    ki = lax.broadcasted_iota(jnp.int32, (32, 48), 1)
    in_a = ki < 40
    ok_a = in_a & ((qi < 8) | (qi >= ki))
    fill_a = jnp.where(in_a, -1e9, -jnp.inf).astype(F32)
    qi = lax.broadcasted_iota(jnp.int32, (48, 80), 0)
    ki = lax.broadcasted_iota(jnp.int32, (48, 80), 1)
    q_first = qi < 8
    q_mem = (qi >= 16) & (qi < 24)
    qtok = jnp.where(qi < 16, qi + 24, qi + 16)
    k_first = ki < 40
    k_mem = (ki < 8) | ((ki >= 48) & (ki < 56))
    ktok = jnp.where(ki < 48, ki - 8, ki - 16)
    in_b = (q_first & k_first) | ((~q_first) & (~k_first))
    ok_b = in_b & (q_mem | k_mem | (qtok >= ktok))
    fill_b = jnp.where(in_b, -1e9, -jnp.inf).astype(F32)
    return ok_a, fill_a, ok_b, fill_b


def _ftile(j):
    return j * 128, min((j + 1) * 128, FH)


def _kernel(x_hbm, mem0_ref, wq_hbm, wk_hbm, wv_hbm, wo_hbm, wint_hbm, wsp_hbm, bsp_ref, wout_hbm,
            out_hbm,
            xbuf, xn, xnb, wraw, wqkv, wo, wint, wsp, wout, z1, z2, bcol, gate, ubuf,
            ka, va, qd, oa, ob, obuf, sems, osem):
    scale = DH ** -0.5
    w32 = [w.bitcast(U32) for w in (wq_hbm, wk_hbm, wv_hbm)]
    x32 = x_hbm.bitcast(U32)
    wsp32 = wsp_hbm.bitcast(U32)

    def cp_rows(src, dst, r0, n, sem):
        return pltpu.make_async_copy(src.at[pl.ds(r0 // 2, n // 2)], dst.at[pl.ds(r0 // 2, n // 2)], sems.at[sem])

    def cp_wpair(J, p):
        return pltpu.make_async_copy(w32[J // 16].at[:, p, J % 16, :], wraw.at[J, p], sems.at[SEM_W + J // JPI])

    x_parts = ((0, 512), (512, 512), (1024, 1024))
    cp_x = [cp_rows(x32, xbuf, r, n, SEM_X + j) for j, (r, n) in enumerate(x_parts)]
    cp_win = pltpu.make_async_copy(wint_hbm.bitcast(U32), wint, sems.at[SEM_WIN])
    cp_wout = pltpu.make_async_copy(wout_hbm.bitcast(U32), wout, sems.at[SEM_WOUT])
    cp_wsp = [cp_rows(wsp32, wsp, m * RB2, RB2, SEM_WSP + m) for m in range(NB2)]
    nA = (WSP_A + 1) * GR
    cp_wspa = cp_rows(wsp32, wsp, R0, nA, SEM_WSP + NB2)
    cp_wspb = cp_rows(wsp32, wsp, R0 + nA, S - R0 - nA, SEM_WSP + NB2 + 1)
    cp_wo = pltpu.make_async_copy(wo_hbm.bitcast(U32), wo, sems.at[SEM_WO])

    def start_group(m):
        for c in [cp_wsp[m]] + [cp_wpair(J, p) for J in range(m * JPI, (m + 1) * JPI) for p in range(2)]:
            c.start()

    for c in [cp_x[0], cp_win, cp_x[1], cp_x[2], cp_wout]:
        c.start()
    start_group(0)

    bsp = bsp_ref[...].astype(F32)
    for c in range(16):
        bcol[c * 128:(c + 1) * 128, :] = jnp.transpose(jnp.broadcast_to(bsp[c:c + 1, :], (128, 128)))

    def ln_x(blk):
        r0 = pl.multiple_of(blk * RB, RB)
        h0 = pl.multiple_of(blk * (RB // 2), RB // 2)
        x = _bf(xbuf[pl.ds(h0, RB // 2), :]).astype(F32)
        m = jnp.mean(x, axis=-1, keepdims=True)
        xc = x - m
        v = jnp.mean(xc * xc, axis=-1, keepdims=True)
        xnv = xc * lax.rsqrt(v + EPS)
        xn[pl.ds(r0, RB), :] = xnv
        xnb[pl.ds(h0, RB // 2), :] = _u32(xnv.astype(BF16))

    def relayout(J):
        for r in range(0, D // 2, 80):
            ev = wraw[J, 0, r:r + 80, :]
            od = wraw[J, 1, r:r + 80, :]
            wqkv[2 * J, r:r + 80, :] = (ev & jnp.uint32(0xFFFF)) | (od << 16)
            wqkv[2 * J + 1, r:r + 80, :] = (ev >> 16) | (od & jnp.uint32(0xFFFF0000))

    cp_x[0].wait()
    ln_x(0)
    cp_win.wait()

    def ph1(i, c):
        @pl.when(i == 1)
        def _():
            start_group(1)
            cp_x[1].wait()

        @pl.when(i == 3)
        def _():
            start_group(2)
            cp_x[2].wait()

        @pl.when(i == 5)
        def _():
            start_group(3)
            for cp in (cp_wo, cp_wspa, cp_wspb):
                cp.start()
        r0 = pl.multiple_of(i * RB, RB)
        h0 = pl.multiple_of(i * (RB // 2), RB // 2)
        xb = _bf(xnb[pl.ds(h0, RB // 2), :])
        zz2 = _gelu(_dot_nt(xb, _bf(wint[FH // 2:FH, :])))
        m2 = jnp.mean(zz2, axis=-1, keepdims=True)
        zc = zz2 - m2
        v2 = jnp.mean(zc * zc, axis=-1, keepdims=True)
        z2[pl.ds(h0, RB // 2), :] = _u32((zc * lax.rsqrt(v2 + EPS)).astype(BF16))
        z1[pl.ds(r0, RB), :] = _dot_nt(xb, _bf(wint[0:FH // 2, :]))
        ln_x(jnp.minimum(i + 1, NB1 - 1))
        return c
    lax.fori_loop(0, NB1, ph1, 0)

    cp_wout.wait()

    def g_unit(g0, nrows, j):
        lo, hi = _ftile(j)
        gh = pl.multiple_of(g0 // 2, 8)
        g = _dot(_bf(wsp[pl.ds(gh, nrows // 2), :]), _bf(z2[:, lo:hi]))
        g = g + bcol[pl.ds(g0, nrows), 0:hi - lo]
        u = (_gelu(z1[pl.ds(g0, nrows), lo:hi]) * g).astype(BF16)
        ubuf[0:nrows // 2, lo:hi] = _u32(u)

    def m_unit(g0, nrows, c):
        gm = _dot(_bf(ubuf[0:nrows // 2, :]), _bf(wout[:, c * 128:(c + 1) * 128]))
        gate[pl.ds(g0, nrows), c * 128:(c + 1) * 128] = gm * jax.nn.sigmoid(gm)

    def ph2(m, c):
        g0 = pl.multiple_of(m * RB2, RB2)
        pltpu.make_async_copy(wsp32.at[pl.ds(0, RB2 // 2)], wsp.at[pl.ds(pl.multiple_of(m * (RB2 // 2), RB2 // 2), RB2 // 2)],
                              sems.at[SEM_WSP + m]).wait()
        wgrp = wraw.at[pl.ds(m * JPI, JPI)]
        pltpu.make_async_copy(wgrp, wgrp, sems.at[SEM_W + m]).wait()
        for j in range(NF):
            g_unit(g0, RB2, j)
            relayout(m * JPI + j)
        for cc in range(5):
            m_unit(g0, RB2, cc)
            relayout(m * JPI + NF + cc)
        return c
    lax.fori_loop(0, NB2, ph2, 0)
    cp_wspa.wait()
    cp_wo.wait()

    sched = {}
    for item in SCHED.split(','):
        k, v = item.split(':')
        sched[k] = [v[n:n + 2] for n in range(0, len(v), 2)]

    for us in sched.values():
        for u in us:
            if u[0] == 'n':
                g_unit(R0, GR, int(u[1]))

    def pair(i, mem):
        @pl.when(i == WSP_A - 1)
        def _():
            cp_wspb.wait()
        ok_a, fill_a, ok_b, fill_b = _masks()
        r0 = pl.multiple_of(i * 64, 64)
        g0 = pl.multiple_of(R0 + i * GR, 16)
        g0n = pl.multiple_of(R0 + jnp.minimum(i + 1, NPAIR - 1) * GR, 16)

        def run_step(hh, first):
            ok, fill = (ok_a, fill_a) if first else (ok_b, fill_b)
            o_ref = oa if first else ob
            name = 'A' if first else 'B'
            st = {}
            acc = [None, 0]

            def wo_chunk(h0, h1):
                part = _dot(_bf(o_ref[:, h0 * 128:h1 * 128]), _bf(wo[h0 * 64:h1 * 64, :]))
                acc[0] = part if acc[0] is None else acc[0] + part
                acc[1] = h1

            def fillers(t):
                for u in sched.get('%s%d' % (name, t), []):
                    n = int(u[1])
                    if u[0] == 'g':
                        g_unit(g0, GR, n)
                    elif u[0] == 'n':
                        g_unit(g0n, GR, n)
                    elif u[0] == 'm':
                        m_unit(g0, GR, n)
                    elif u[0] == 'w':
                        wo_chunk(acc[1], acc[1] + 4)

            for t in range(H + SK_PV + 1):
                if t < H:
                    h = t
                    w = jnp.concatenate([wqkv[h], wqkv[H + h], wqkv[2 * H + h]], axis=1)
                    qkv = _dot(hh, _bf(w))
                    q = qkv[:, 0:128].astype(BF16)
                    k = qkv[:, 128:256].astype(BF16)
                    v = qkv[:, 256:384].astype(BF16)
                    if first:
                        ka[h] = _u32(k)
                        va[h] = _u32(v)
                        qd[h] = _u32(q[32:48])
                        q = q[0:32]
                    st[h] = (q, k, v)
                fillers(t)
                h = t - SK_S
                if 0 <= h < H:
                    q, k, v = st[h]
                    if not first:
                        q = jnp.concatenate([_bf(qd[h]), q], axis=0)
                        k = jnp.concatenate([_bf(ka[h]), k], axis=0)
                    s = _dot_nt(q, k)
                    s = jnp.where(ok, s * scale, fill)
                    mx = jnp.max(s, axis=-1, keepdims=True)
                    e = jnp.exp(s - mx)
                    l = jnp.sum(e, axis=-1, keepdims=True)
                    st[h] = ((e * (1.0 / l)).astype(BF16), v)
                h = t - SK_PV
                if 0 <= h < H:
                    p, v = st.pop(h)
                    if not first:
                        v = jnp.concatenate([_bf(va[h]), v], axis=0)
                    o = _dot(p, v)
                    o_ref[:, h * 128:(h + 1) * 128] = _u32(o.astype(BF16))
            wo_chunk(acc[1], H)
            res = acc[0]
            return res, (lambda: fillers(99))

        ha = jnp.concatenate([mem, xn[pl.ds(r0, 40), :]], axis=0).astype(BF16)
        sa, f99 = run_step(ha, True)
        f99()
        mem = sa[0:8]
        hb = jnp.concatenate([mem, xn[pl.ds(r0 + 40, 24), :]], axis=0).astype(BF16)
        sb, f99 = run_step(hb, False)
        f99()
        mem = sb[16:24]
        sall = jnp.concatenate([sa[8:32], sb[0:16], sb[24:48]], axis=0)
        obuf[pl.ds(r0, 64), :] = (_bf(xbuf[pl.ds(pl.multiple_of(i * 32, 32), 32), :]).astype(F32) + sall * gate[pl.ds(r0, 64), :]).astype(BF16)
        pltpu.make_async_copy(obuf.at[pl.ds(r0, 64), :], out_hbm.at[pl.ds(r0, 64), :], osem).start()
        return mem

    lax.fori_loop(0, NPAIR, pair, mem0_ref[...].astype(F32))
    pltpu.make_async_copy(obuf, out_hbm, osem).wait()


@functools.partial(jax.jit, static_argnames=("A_seg_len",))
def pallas_recurrent_scan__memory_aug_recurrent_mem_tr__mixer_gmlp__prompt_kernel(A_x, A_mem0, A_Wq, A_Wk, A_Wv, A_Wo, A_seg_len, B_x, B_w_in, B_w_sp, B_b_sp, B_w_out):
    any_spec = pl.BlockSpec(memory_space=pl.ANY)
    vmem_spec = pl.BlockSpec(memory_space=pltpu.VMEM)
    out = pl.pallas_call(
        _kernel,
        out_shape=jax.ShapeDtypeStruct((S, D), BF16),
        in_specs=[any_spec, vmem_spec, any_spec, any_spec, any_spec, any_spec, any_spec, any_spec, vmem_spec, any_spec],
        out_specs=any_spec,
        scratch_shapes=[
            pltpu.VMEM((S // 2, D), U32),
            pltpu.VMEM((S, D), F32),
            pltpu.VMEM((S // 2, D), U32),
            pltpu.VMEM((NJ, 2, D // 2, DH), U32),
            pltpu.VMEM((3 * H, D // 2, DH), U32),
            pltpu.VMEM((H * DH // 2, D), U32),
            pltpu.VMEM((FH, D), U32),
            pltpu.VMEM((S // 2, S), U32),
            pltpu.VMEM((FH // 2, D), U32),
            pltpu.VMEM((S, FH), F32),
            pltpu.VMEM((S // 2, FH), U32),
            pltpu.VMEM((S, 128), F32),
            pltpu.VMEM((S, D), F32),
            pltpu.VMEM((64, FH), U32),
            pltpu.VMEM((H, 24, DH), U32),
            pltpu.VMEM((H, 24, DH), U32),
            pltpu.VMEM((H, 8, DH), U32),
            pltpu.VMEM((16, H * DH), U32),
            pltpu.VMEM((24, H * DH), U32),
            pltpu.VMEM((S, D), BF16),
            pltpu.SemaphoreType.DMA((NSEM,)),
            pltpu.SemaphoreType.DMA,
        ],
        compiler_params=pltpu.CompilerParams(vmem_limit_bytes=110 * 1024 * 1024),
    )(A_x.reshape(S, D), A_mem0.reshape(M, D), A_Wq.reshape(D // 2, 2, H, DH), A_Wk.reshape(D // 2, 2, H, DH), A_Wv.reshape(D // 2, 2, H, DH), A_Wo.reshape(H * DH, D),
      B_w_in.T, B_w_sp, B_b_sp.reshape(16, 128), B_w_out)
    return out.reshape(1, S, D)
```

```python
import functools
import jax
import jax.numpy as jnp
from jax import lax
import jax.experimental.pallas as pl
import jax.experimental.pallas.tpu as pltpu

F32 = jnp.float32
BF16 = jnp.bfloat16
U32 = jnp.uint32

S, D, H, DH, M, SEG = 2048, 640, 32, 128, 8, 32
FH = 864
FF = 768
FR = FH - FF
NFT = FF // 128
NPAIR = S // (2 * SEG)
UNR = 2
NBODY = NPAIR // UNR
EPS = 1e-5
SUB = 128
NBLK = S // SUB
R0 = 1024
GR = (S - R0) // NBODY
P1B = 2
P2B = 2
SKA_S, SKA_PV, SKB_S, SKB_PV = 2, 5, 2, 5
SCHED = (
    'A32:g1,A33:w0,A34:w0,A35:w0,A36:w0,A99:g2,B32:g3,B33:w0,B34:w0,B35:w0,B36:w0,B99:g4;'
    'A32:g5,A33:w0,A34:w0,A35:w0,A36:w0,A99:m0m1,B32:m2m3,B33:m4,B34:w0,B35:w0,B36:w0,B99:n0')

NJ = 3 * H // 2
N1 = (NBLK - 4) // P1B
N2 = (R0 // SUB) // P2B
JP1 = 4
JP2 = (NJ - N1 * JP1) // N2
assert N1 * JP1 + N2 * JP2 == NJ
SEM_X = 0
SEM_WIN = 8
SEM_W = 11
SEM_WOUT = SEM_W + N1 + N2
SEM_WSP = SEM_WOUT + 1
SEM_WO = SEM_WSP + N2
SEM_SMALL = SEM_WO + 1
NSEM = SEM_SMALL + 2


def _bf(x):
    return pltpu.bitcast(x, BF16)


def _u32(x):
    return pltpu.bitcast(x, U32)


def _dot(a, b):
    return jnp.dot(a, b, preferred_element_type=F32)


def _dot_nt(a, b):
    return lax.dot_general(a, b, (((1,), (1,)), ((), ())), preferred_element_type=F32)


def _gelu(x):
    c = 0.7978845608028654
    t = jnp.tanh(x * (c + (c * 0.044715) * (x * x)))
    hx = 0.5 * x
    return hx + hx * t


def _masks():
    qi = lax.broadcasted_iota(jnp.int32, (32, 48), 0)
    ki = lax.broadcasted_iota(jnp.int32, (32, 48), 1)
    in_a = ki < 40
    ok_a = in_a & ((qi < 8) | (qi >= ki))
    fill_a = jnp.where(in_a, -1e9, -jnp.inf).astype(F32)
    qi = lax.broadcasted_iota(jnp.int32, (48, 80), 0)
    ki = lax.broadcasted_iota(jnp.int32, (48, 80), 1)
    q_first = qi < 8
    q_mem = (qi >= 16) & (qi < 24)
    qtok = jnp.where(qi < 16, qi + 24, qi + 16)
    k_first = ki < 40
    k_mem = (ki < 8) | ((ki >= 48) & (ki < 56))
    ktok = jnp.where(ki < 48, ki - 8, ki - 16)
    in_b = (q_first & k_first) | ((~q_first) & (~k_first))
    ok_b = in_b & (q_mem | k_mem | (qtok >= ktok))
    fill_b = jnp.where(in_b, -1e9, -jnp.inf).astype(F32)
    return ok_a, fill_a, ok_b, fill_b


def _kernel(x_hbm, mem0_hbm, wq_hbm, wk_hbm, wv_hbm, wo_hbm, wint_hbm, wsp_hbm, bsp_hbm, wout_hbm,
            out_hbm,
            xbuf, xn, xnb, wraw, wqkv, wo, wint, wsp, wout, z1, z1rt, z2, z2rt, ztmp, bcol, brow, gate, ubuf, urem,
            ka, va, oa, ob, obuf, mem0_ref, bsp_ref, sems, osem):
    scale = DH ** -0.5
    w32 = [w.bitcast(U32) for w in (wq_hbm, wk_hbm, wv_hbm)]
    x32 = x_hbm.bitcast(U32)
    wsp32 = wsp_hbm.bitcast(U32)
    wint32 = wint_hbm.bitcast(U32)

    def cp_rows(src, dst, r0, n, sem):
        return pltpu.make_async_copy(src.at[pl.ds(r0 // 2, n // 2)], dst.at[pl.ds(r0 // 2, n // 2)], sems.at[sem])

    def wait_rows(dst, r0, n, sem):
        d = dst.at[pl.ds(pl.multiple_of(r0 // 2, 8), n // 2)]
        pltpu.make_async_copy(d, d, sems.at[sem]).wait()

    def wgroup(k):
        j0, n = (k * JP1, JP1) if k < N1 else (N1 * JP1 + (k - N1) * JP2, JP2)
        return [pltpu.make_async_copy(w32[J // 16].at[:, p, J % 16, :], wraw.at[J, p], sems.at[SEM_W + k])
                for J in range(j0, j0 + n) for p in range(2)]

    def wait_wgroup(k, j0, n):
        wgrp = wraw.at[pl.ds(j0, n)]
        pltpu.make_async_copy(wgrp, wgrp, sems.at[SEM_W + k]).wait()

    cp_x = [cp_rows(x32, xbuf, j * 256, 256, SEM_X + j) for j in range(8)]
    cp_win = [cp_rows(wint32, wint, FH, 512, SEM_WIN), cp_rows(wint32, wint, FH + 512, FH - 512, SEM_WIN + 1),
              cp_rows(wint32, wint, FF, FR, SEM_WIN + 1), cp_rows(wint32, wint, 0, FF, SEM_WIN + 2)]
    cp_wout = pltpu.make_async_copy(wout_hbm.bitcast(U32), wout, sems.at[SEM_WOUT])
    WSPR = S // N2
    cp_wsp = [cp_rows(wsp32, wsp, m * WSPR, WSPR, SEM_WSP + m) for m in range(N2)]
    cp_wo = pltpu.make_async_copy(wo_hbm.bitcast(U32), wo, sems.at[SEM_WO])

    cp_bsp = pltpu.make_async_copy(bsp_hbm, bsp_ref, sems.at[SEM_SMALL])
    cp_mem0 = pltpu.make_async_copy(mem0_hbm, mem0_ref, sems.at[SEM_SMALL + 1])
    dma = [cp_bsp, cp_x[0], cp_win[0], cp_x[1], cp_mem0, cp_win[1], cp_win[2], cp_win[3], cp_x[2]]
    xs_left = cp_x[3:]
    for k in range(N1):
        for _ in range(P1B // 2 if P1B >= 2 else 1):
            if xs_left:
                dma.append(xs_left.pop(0))
        dma += wgroup(k)
    dma += xs_left + [cp_wout]
    for m in range(N2):
        dma += [cp_wsp[m]] + wgroup(N1 + m)
        if m == N2 - 2:
            dma.append(cp_wo)
    nb = -(-len(dma) // 4)
    batches = [dma[b * nb:(b + 1) * nb] for b in range(4)]

    def start_all(cps):
        for c in cps:
            c.start()

    start_all(batches[0])

    cp_bsp.wait()
    bsp = bsp_ref[...].astype(F32)
    brow[...] = bsp
    for c in range(16):
        bcol[c * 128:(c + 1) * 128, :] = jnp.transpose(jnp.broadcast_to(bsp[c:c + 1, :], (128, 128)))

    def ln_passes(ld, fin):
        st = {}

        def p0():
            st['m'] = jnp.mean(ld(), axis=-1, keepdims=True)

        def p1():
            c = ld() - st['m']
            st['r'] = lax.rsqrt(jnp.mean(c * c, axis=-1, keepdims=True) + EPS)

        def p2():
            fin((ld() - st['m']) * st['r'])
        return [p0, p1, p2]

    def ln_x(b, s):
        r0 = pl.multiple_of(b * SUB, SUB)
        h0 = pl.multiple_of(b * (SUB // 2), SUB // 2)

        def fin(v):
            xn[pl.ds(r0, SUB), :] = v
            xnb[s] = _u32(v.astype(BF16))
        return ln_passes(lambda: _bf(xbuf[pl.ds(h0, SUB // 2), :]).astype(F32), fin)

    def relayout(J):
        for r in range(0, D // 2, 80):
            ev = wraw[J, 0, r:r + 80, :]
            od = wraw[J, 1, r:r + 80, :]
            wqkv[2 * J, r:r + 80, :] = (ev & jnp.uint32(0xFFFF)) | (od << 16)
            wqkv[2 * J + 1, r:r + 80, :] = (ev >> 16) | (od & jnp.uint32(0xFFFF0000))

    def z2_tiles(b, s):
        def tile(j):
            lo = (FH + j * 128) // 2
            ztmp[s, :, j * 128:(j + 1) * 128] = _gelu(_dot_nt(_bf(xnb[s]), _bf(wint[lo:lo + 64, :])))

        def rem():
            wr = jnp.concatenate([wint[FF // 2:FH // 2, :], wint[(FH + FF) // 2:FH, :]], axis=0)
            zr = _dot_nt(_bf(wr), _bf(xnb[s]))
            z1rt[b] = zr[0:FR]
            ztmp[s, :, FF:FH] = jnp.transpose(_gelu(zr[FR:2 * FR]))
        return [functools.partial(tile, j) for j in range(4)] + [rem] + [functools.partial(tile, j) for j in range(4, NFT)]

    def z2_post(b, s):
        def fin(v):
            z2[pl.ds(pl.multiple_of(b * (SUB // 2), SUB // 2), SUB // 2), :] = _u32(v[:, 0:FF].astype(BF16))
            z2rt[b] = _u32(jnp.transpose(v[:, FF:FH]).astype(BF16))
        return ln_passes(lambda: ztmp[s], fin)

    def z1_tiles(b, s):
        r0 = pl.multiple_of(b * SUB, SUB)

        def tile(j):
            z1[pl.ds(r0, SUB), j * 128:(j + 1) * 128] = _dot_nt(_bf(xnb[s]), _bf(wint[j * 64:(j + 1) * 64, :]))
        return [functools.partial(tile, j) for j in range(NFT)]

    def weave(tiles, *passes):
        for n, t in enumerate(tiles):
            t()
            if n % 2 == 0 and n // 2 < 3:
                for p in passes:
                    p[n // 2]()

    cp_x[0].wait()
    for p in ln_x(0, 0) + ln_x(1, 1):
        p()
    cp_win[0].wait()
    t0, t1 = z2_tiles(0, 0), z2_tiles(1, 1)
    weave(t0[0:4] + t1[0:4])
    start_all(batches[1])
    cp_x[1].wait()
    cp_win[1].wait()
    cp_win[2].wait()
    weave(t0[4:] + t1[4:], ln_x(2, 2), ln_x(3, 3))
    weave(z2_tiles(2, 2), z2_post(0, 0))
    weave(z2_tiles(3, 3), z2_post(1, 1))
    cp_win[3].wait()
    cp_x[2].wait()
    weave(z1_tiles(0, 0), z2_post(2, 2))
    weave(z1_tiles(1, 1), z2_post(3, 3))
    weave(z1_tiles(2, 2), ln_x(4, 0))
    weave(z1_tiles(3, 3))

    def ph1(i, c):
        @pl.when(i == N1 // 3)
        def _():
            start_all(batches[2])

        @pl.when(i == (2 * N1) // 3)
        def _():
            start_all(batches[3])
        b0 = 4 + i * P1B
        for u in range(max(P1B // 2, 1)):
            ch = (b0 + 2) // 2 + u

            @pl.when(ch < 8)
            def _():
                wait_rows(xbuf, ch * 256, 256, SEM_X + ch)
        wait_wgroup(i, i * JP1, JP1)
        for u in range(P1B):
            b = b0 + u
            bn = jnp.minimum(b + 1, NBLK - 1)
            weave(z2_tiles(b, u), ln_x(bn, (u + 1) % P1B))
            weave(z1_tiles(b, u), z2_post(b, u))
        for jj in range(JP1):
            relayout(i * JP1 + jj)
        return c
    lax.fori_loop(0, N1, ph1, 0)

    cp_wout.wait()

    def g_unit(g0, nrows, j):
        gh = pl.multiple_of(g0 // 2, 8)
        g = _dot(_bf(wsp[pl.ds(gh, nrows // 2), :]), _bf(z2[:, j * 128:(j + 1) * 128]))
        g = g + bcol[pl.ds(g0, nrows), :]
        u = (_gelu(z1[pl.ds(g0, nrows), j * 128:(j + 1) * 128]) * g).astype(BF16)
        ubuf[0:nrows // 2, j * 128:(j + 1) * 128] = _u32(u)

    def r_unit(b):
        h0 = pl.multiple_of(b * (SUB // 2), SUB // 2)
        lhs = jnp.concatenate([z2rt[k] for k in range(NBLK)], axis=1)
        gt = _dot_nt(_bf(lhs), _bf(wsp[pl.ds(h0, SUB // 2), :]))
        ut = _gelu(z1rt[b]) * (gt + brow[pl.ds(b, 1), :])
        urem[pl.ds(h0, SUB // 2), :] = _u32(jnp.transpose(ut).astype(BF16))

    def m_unit(g0, nrows, c):
        gh = pl.multiple_of(g0 // 2, 8)
        u = jnp.concatenate([ubuf[0:nrows // 2, :], urem[pl.ds(gh, nrows // 2), :]], axis=1)
        gm = _dot(_bf(u), _bf(wout[:, c * 128:(c + 1) * 128]))
        gate[pl.ds(g0, nrows), c * 128:(c + 1) * 128] = gm * jax.nn.sigmoid(gm)

    def ph2(m, c):
        wait_rows(wsp, m * WSPR, WSPR, SEM_WSP + m)
        j0 = N1 * JP1 + m * JP2
        wait_wgroup(N1 + m, j0, JP2)
        nr = P2B * SUB
        g0 = pl.multiple_of(m * nr, nr)
        rb = [m * 2 * P2B + u for u in range(2 * P2B)]
        for j in range(NFT):
            g_unit(g0, nr, j)
            if j < len(rb):
                r_unit(rb[j])
        for cc in range(5):
            m_unit(g0, nr, cc)
        for jj in range(JP2):
            relayout(j0 + jj)
        return c
    lax.fori_loop(0, N2, ph2, 0)
    cp_wo.wait()
    cp_mem0.wait()

    scheds = []
    for part in SCHED.split(';'):
        sched = {}
        for item in part.split(','):
            k, v = item.split(':')
            sched[k] = [v[n:n + 2] for n in range(0, len(v), 2)]
        scheds.append(sched)

    for sched in scheds:
        for us in sched.values():
            for u in us:
                if u[0] == 'n':
                    g_unit(R0, GR, int(u[1]))

    def pair(i, mem, sched, g0, g0n):
        ok_a, fill_a, ok_b, fill_b = _masks()
        r0 = pl.multiple_of(i * 64, 64)

        def run_step(hq, hh, first):
            ok, fill = (ok_a, fill_a) if first else (ok_b, fill_b)
            o_ref = oa if first else ob
            name = 'A' if first else 'B'
            st = {}
            acc = [None, 0]

            def wo_chunk(h0, h1):
                part = _dot(_bf(o_ref[:, h0 * 128:h1 * 128]), _bf(wo[h0 * 64:h1 * 64, :]))
                acc[0] = part if acc[0] is None else acc[0] + part
                acc[1] = h1

            def fillers(t):
                for u in sched.get('%s%d' % (name, t), []):
                    n = int(u[1])
                    if u[0] == 'g':
                        g_unit(g0, GR, n)
                    elif u[0] == 'n':
                        g_unit(g0n, GR, n)
                    elif u[0] == 'm':
                        m_unit(g0, GR, n)
                    elif u[0] == 'w':
                        wo_chunk(acc[1], acc[1] + 4)

            SK_S, SK_PV = (SKA_S, SKA_PV) if first else (SKB_S, SKB_PV)

            def do_s(h):
                q, k, v = st[h]
                if not first:
                    k = jnp.concatenate([_bf(ka[h]), k], axis=0)
                s = _dot_nt(q, k)
                s = jnp.where(ok, s * scale, fill)
                mx = jnp.max(s, axis=-1, keepdims=True)
                e = jnp.exp(s - mx)
                l = jnp.sum(e, axis=-1, keepdims=True)
                r = pl.reciprocal(l, approx=True)
                r = r * (2.0 - l * r)
                st[h] = ((e * r).astype(BF16), v)

            def do_pv(h):
                p, v = st.pop(h)
                if not first:
                    v = jnp.concatenate([_bf(va[h]), v], axis=0)
                o = _dot(p, v)
                o_ref[:, h * 128:(h + 1) * 128] = _u32(o.astype(BF16))

            for t in range(H + SK_PV + 1):
                if t < H:
                    h = t
                    q = _dot(hq, _bf(wqkv[h])).astype(BF16)
                    kv = _dot(hh, _bf(jnp.concatenate([wqkv[H + h], wqkv[2 * H + h]], axis=1)))
                    k = kv[:, 0:128].astype(BF16)
                    v = kv[:, 128:256].astype(BF16)
                    if first:
                        ka[h] = _u32(k)
                        va[h] = _u32(v)
                    st[h] = (q, k, v)
                fillers(t)
                if 0 <= t - SK_PV < H:
                    do_pv(t - SK_PV)
                if 0 <= t - SK_S < H:
                    do_s(t - SK_S)
            wo_chunk(acc[1], H)
            res = acc[0]
            fillers(99)
            return res

        ha = jnp.concatenate([mem, xn[pl.ds(r0, 40), :]], axis=0).astype(BF16)
        sa = run_step(ha[0:32], ha, True)
        mem = sa[0:8]
        hb = jnp.concatenate([mem, xn[pl.ds(r0 + 40, 24), :]], axis=0).astype(BF16)
        sb = run_step(jnp.concatenate([ha[32:48], hb], axis=0), hb, False)
        mem = sb[16:24]
        sall = jnp.concatenate([sa[8:32], sb[0:16], sb[24:48]], axis=0)
        xr = _bf(xbuf[pl.ds(pl.multiple_of(i * 32, 32), 32), :]).astype(F32)
        obuf[pl.ds(r0, 64), :] = (xr + sall * gate[pl.ds(r0, 64), :]).astype(BF16)
        return mem

    def body(ii, mem):
        g0 = pl.multiple_of(R0 + ii * GR, 16)
        g0n = pl.multiple_of(R0 + jnp.minimum(ii + 1, NBODY - 1) * GR, 16)
        for u in range(UNR):
            mem = pair(ii * UNR + u, mem, scheds[u], g0, g0n)
        r0 = pl.multiple_of(ii * (64 * UNR), 64 * UNR)
        pltpu.make_async_copy(obuf.at[pl.ds(r0, 64 * UNR), :], out_hbm.at[pl.ds(r0, 64 * UNR), :], osem).start()
        return mem

    lax.fori_loop(0, NBODY, body, mem0_ref[...].astype(F32))
    pltpu.make_async_copy(obuf, out_hbm, osem).wait()


@functools.partial(jax.jit, static_argnames=("A_seg_len",))
def pallas_recurrent_scan__memory_aug_recurrent_mem_tr__mixer_gmlp__prompt_kernel(A_x, A_mem0, A_Wq, A_Wk, A_Wv, A_Wo, A_seg_len, B_x, B_w_in, B_w_sp, B_b_sp, B_w_out):
    any_spec = pl.BlockSpec(memory_space=pl.ANY)
    vmem_spec = pl.BlockSpec(memory_space=pltpu.VMEM)
    out = pl.pallas_call(
        _kernel,
        out_shape=jax.ShapeDtypeStruct((S, D), BF16),
        in_specs=[any_spec] * 10,
        out_specs=any_spec,
        scratch_shapes=[
            pltpu.VMEM((S // 2, D), U32),
            pltpu.VMEM((S, D), F32),
            pltpu.VMEM((4, SUB // 2, D), U32),
            pltpu.VMEM((NJ, 2, D // 2, DH), U32),
            pltpu.VMEM((3 * H, D // 2, DH), U32),
            pltpu.VMEM((H * DH // 2, D), U32),
            pltpu.VMEM((FH, D), U32),
            pltpu.VMEM((S // 2, S), U32),
            pltpu.VMEM((FH // 2, D), U32),
            pltpu.VMEM((S, FF), F32),
            pltpu.VMEM((NBLK, FR, SUB), F32),
            pltpu.VMEM((S // 2, FF), U32),
            pltpu.VMEM((NBLK, FR // 2, SUB), U32),
            pltpu.VMEM((4, SUB, FH), F32),
            pltpu.VMEM((S, 128), F32),
            pltpu.VMEM((16, 128), F32),
            pltpu.VMEM((S, D), F32),
            pltpu.VMEM((P2B * SUB // 2, FF), U32),
            pltpu.VMEM((S // 2, FR), U32),
            pltpu.VMEM((H, 24, DH), U32),
            pltpu.VMEM((H, 24, DH), U32),
            pltpu.VMEM((16, H * DH), U32),
            pltpu.VMEM((24, H * DH), U32),
            pltpu.VMEM((S, D), BF16),
            pltpu.VMEM((M, D), BF16),
            pltpu.VMEM((16, 128), BF16),
            pltpu.SemaphoreType.DMA((NSEM,)),
            pltpu.SemaphoreType.DMA,
        ],
        compiler_params=pltpu.CompilerParams(vmem_limit_bytes=110 * 1024 * 1024),
    )(A_x.reshape(S, D), A_mem0.reshape(M, D), A_Wq.reshape(D // 2, 2, H, DH), A_Wk.reshape(D // 2, 2, H, DH),
      A_Wv.reshape(D // 2, 2, H, DH), A_Wo.reshape(H * DH, D),
      B_w_in.T, B_w_sp, B_b_sp.reshape(16, 128), B_w_out)
    return out.reshape(1, S, D)
```

```python
import functools
import jax
import jax.numpy as jnp
from jax import lax
import jax.experimental.pallas as pl
import jax.experimental.pallas.tpu as pltpu

F32 = jnp.float32
BF16 = jnp.bfloat16
U32 = jnp.uint32

S, D, H, DH, M, SEG = 2048, 640, 32, 128, 8, 32
FH = 864
FF = 768
FR = FH - FF
NFT = FF // 128
NPAIR = S // (2 * SEG)
UNR = 2
NBODY = NPAIR // UNR
EPS = 1e-5
SUB = 128
NBLK = S // SUB
R0 = 1024
GR = (S - R0) // NBODY
P1B = 2
P2B = 2
SKA_S, SKA_PV, SKB_S, SKB_PV = 2, 5, 2, 7
SCHED = (
    'A32:g1,A33:w0,A34:w0,A35:w0,A36:w0,A99:g2,B32:g3,B33:w0,B34:w0,B35:w0,B36:w0,B99:g4;'
    'A32:g5,A33:w0,A34:w0,A35:w0,A36:w0,A99:m0m1,B32:m2m3,B33:m4,B34:w0,B35:w0,B36:w0,B99:n0')

SK_VA = 2
SK_VB = 2
LOG2E = 1.4426950408889634
DV = -3
DE = 0
TOKA = 2
TOKB = 3
TOKREV = 0
NJ = 3 * H // 2
N1 = (NBLK - 4) // P1B
N2 = (R0 // SUB) // P2B
JP1 = 4
JP2 = (NJ - N1 * JP1) // N2
assert N1 * JP1 + N2 * JP2 == NJ
NA = 2 * N1 * JP1
assert NA >= H
SEM_X = 0
SEM_WIN = 8
SEM_W = 11
SEM_WOUT = SEM_W + N1 + N2
SEM_WSP = SEM_WOUT + 1
SEM_WO = SEM_WSP + N2
SEM_SMALL = SEM_WO + 1
NSEM = SEM_SMALL + 2


def _bf(x):
    return pltpu.bitcast(x, BF16)


def _u32(x):
    return pltpu.bitcast(x, U32)


def _dot(a, b):
    return jnp.dot(a, b, preferred_element_type=F32)


def _dot_nt(a, b):
    return lax.dot_general(a, b, (((1,), (1,)), ((), ())), preferred_element_type=F32)


def _gelu(x):
    c = 0.7978845608028654
    t = jnp.tanh(x * (c + (c * 0.044715) * (x * x)))
    hx = 0.5 * x
    return hx + hx * t


def _tree(op, xs):
    xs = list(xs)
    while len(xs) > 1:
        xs = [op(xs[n], xs[n + 1]) if n + 1 < len(xs) else xs[n] for n in range(0, len(xs), 2)]
    return xs[0]


def _mask():
    qi = lax.broadcasted_iota(jnp.int32, (32, 40), 0)
    ki = lax.broadcasted_iota(jnp.int32, (32, 40), 1)
    return (qi < 8) | (ki < 8) | (ki >= 32) | (qi >= ki)


def _kernel(x_hbm, mem0_hbm, wq_hbm, wk_hbm, wv_hbm, wo_hbm, wint_hbm, wsp_hbm, bsp_hbm, wout_hbm,
            out_hbm,
            xbuf, xn, xnb, wraw, wa, wb, wo, wint, wsp, wout, z1, z1rt, z2, z2rt, ztmp, bcol, brow, gate, ubuf, urem,
            kvf, qs, oa, ob, obuf, mem0_ref, bsp_ref, sems, osem):
    scale = DH ** -0.5
    w32 = [w.bitcast(U32) for w in (wq_hbm, wk_hbm, wv_hbm)]
    x32 = x_hbm.bitcast(U32)
    wsp32 = wsp_hbm.bitcast(U32)
    wint32 = wint_hbm.bitcast(U32)

    def cp_rows(src, dst, r0, n, sem):
        return pltpu.make_async_copy(src.at[pl.ds(r0 // 2, n // 2)], dst.at[pl.ds(r0 // 2, n // 2)], sems.at[sem])

    def wait_rows(dst, r0, n, sem):
        d = dst.at[pl.ds(pl.multiple_of(r0 // 2, 8), n // 2)]
        pltpu.make_async_copy(d, d, sems.at[sem]).wait()

    def wgroup(k):
        j0, n = (k * JP1, JP1) if k < N1 else (N1 * JP1 + (k - N1) * JP2, JP2)
        return [pltpu.make_async_copy(w32[J // 16].at[:, p, J % 16, :], wraw.at[J, p], sems.at[SEM_W + k])
                for J in range(j0, j0 + n) for p in range(2)]

    def wait_wgroup(k, j0, n):
        wgrp = wraw.at[pl.ds(j0, n)]
        pltpu.make_async_copy(wgrp, wgrp, sems.at[SEM_W + k]).wait()

    cp_x = [cp_rows(x32, xbuf, j * 256, 256, SEM_X + j) for j in range(8)]
    cp_win = [cp_rows(wint32, wint, FH, 512, SEM_WIN), cp_rows(wint32, wint, FH + 512, FH - 512, SEM_WIN + 1),
              cp_rows(wint32, wint, FF, FR, SEM_WIN + 1), cp_rows(wint32, wint, 0, FF, SEM_WIN + 2)]
    cp_wout = pltpu.make_async_copy(wout_hbm.bitcast(U32), wout, sems.at[SEM_WOUT])
    WSPR = S // N2
    cp_wsp = [cp_rows(wsp32, wsp, m * WSPR, WSPR, SEM_WSP + m) for m in range(N2)]
    cp_wo = pltpu.make_async_copy(wo_hbm.bitcast(U32), wo, sems.at[SEM_WO])

    cp_bsp = pltpu.make_async_copy(bsp_hbm, bsp_ref, sems.at[SEM_SMALL])
    cp_mem0 = pltpu.make_async_copy(mem0_hbm, mem0_ref, sems.at[SEM_SMALL + 1])
    dma = [cp_bsp, cp_x[0], cp_win[0], cp_x[1], cp_mem0, cp_win[1], cp_win[2], cp_win[3], cp_x[2]]
    xs_left = cp_x[3:]
    for k in range(N1):
        for _ in range(P1B // 2 if P1B >= 2 else 1):
            if xs_left:
                dma.append(xs_left.pop(0))
        dma += wgroup(k)
    dma += xs_left + [cp_wout]
    for m in range(N2):
        dma += [cp_wsp[m]] + wgroup(N1 + m)
        if m == N2 - 2:
            dma.append(cp_wo)
    nb = -(-len(dma) // 4)
    batches = [dma[b * nb:(b + 1) * nb] for b in range(4)]

    def start_all(cps):
        for c in cps:
            c.start()

    start_all(batches[0])

    cp_bsp.wait()
    bsp = bsp_ref[...].astype(F32)
    brow[...] = bsp
    kvf[:, 0:16, :] = jnp.zeros((H, 16, DH), F32)
    for c in range(16):
        bcol[c * 128:(c + 1) * 128, :] = jnp.transpose(jnp.broadcast_to(bsp[c:c + 1, :], (128, 128)))

    def ln_passes(ld, fin):
        st = {}

        def p0():
            st['m'] = jnp.mean(ld(), axis=-1, keepdims=True)

        def p1():
            c = ld() - st['m']
            st['r'] = lax.rsqrt(jnp.mean(c * c, axis=-1, keepdims=True) + EPS)

        def p2():
            fin((ld() - st['m']) * st['r'])
        return [p0, p1, p2]

    def ln_x(b, s):
        r0 = pl.multiple_of(b * SUB, SUB)
        h0 = pl.multiple_of(b * (SUB // 2), SUB // 2)

        def fin(v):
            xn[pl.ds(r0, SUB), :] = v
            xnb[s] = _u32(v.astype(BF16))
        return ln_passes(lambda: _bf(xbuf[pl.ds(h0, SUB // 2), :]).astype(F32), fin)

    def relayout(J, dst, j0):
        for r in range(0, D // 2, 80):
            ev = wraw[J, 0, r:r + 80, :]
            od = wraw[J, 1, r:r + 80, :]
            dst[2 * (J - j0), r:r + 80, :] = (ev & jnp.uint32(0xFFFF)) | (od << 16)
            dst[2 * (J - j0) + 1, r:r + 80, :] = (ev >> 16) | (od & jnp.uint32(0xFFFF0000))

    def wslab(n):
        return wa[n] if n < NA else wb[n - NA]

    def z2_tiles(b, s):
        def tile(j):
            lo = (FH + j * 128) // 2
            ztmp[s, :, j * 128:(j + 1) * 128] = _gelu(_dot_nt(_bf(xnb[s]), _bf(wint[lo:lo + 64, :])))

        def rem():
            wr = jnp.concatenate([wint[FF // 2:FH // 2, :], wint[(FH + FF) // 2:FH, :]], axis=0)
            zr = _dot_nt(_bf(wr), _bf(xnb[s]))
            z1rt[b] = zr[0:FR]
            ztmp[s, :, FF:FH] = jnp.transpose(_gelu(zr[FR:2 * FR]))
        return [functools.partial(tile, j) for j in range(4)] + [rem] + [functools.partial(tile, j) for j in range(4, NFT)]

    def z2_post(b, s):
        def fin(v):
            z2[pl.ds(pl.multiple_of(b * (SUB // 2), SUB // 2), SUB // 2), :] = _u32(v[:, 0:FF].astype(BF16))
            z2rt[b] = _u32(jnp.transpose(v[:, FF:FH]).astype(BF16))
        return ln_passes(lambda: ztmp[s], fin)

    def z1_tiles(b, s):
        r0 = pl.multiple_of(b * SUB, SUB)

        def tile(j):
            z1[pl.ds(r0, SUB), j * 128:(j + 1) * 128] = _dot_nt(_bf(xnb[s]), _bf(wint[j * 64:(j + 1) * 64, :]))
        return [functools.partial(tile, j) for j in range(NFT)]

    def weave(tiles, *passes):
        for n, t in enumerate(tiles):
            t()
            if n % 2 == 0 and n // 2 < 3:
                for p in passes:
                    p[n // 2]()

    cp_x[0].wait()
    for p in ln_x(0, 0) + ln_x(1, 1):
        p()
    cp_win[0].wait()
    t0, t1 = z2_tiles(0, 0), z2_tiles(1, 1)
    weave(t0[0:4] + t1[0:4])
    start_all(batches[1])
    cp_x[1].wait()
    cp_win[1].wait()
    cp_win[2].wait()
    weave(t0[4:] + t1[4:], ln_x(2, 2), ln_x(3, 3))
    weave(z2_tiles(2, 2), z2_post(0, 0))
    weave(z2_tiles(3, 3), z2_post(1, 1))
    cp_win[3].wait()
    cp_x[2].wait()
    weave(z1_tiles(0, 0), z2_post(2, 2))
    weave(z1_tiles(1, 1), z2_post(3, 3))
    weave(z1_tiles(2, 2), ln_x(4, 0))
    weave(z1_tiles(3, 3))

    def ph1(i, c):
        @pl.when(i == N1 // 3)
        def _():
            start_all(batches[2])

        @pl.when(i == (2 * N1) // 3)
        def _():
            start_all(batches[3])
        b0 = 4 + i * P1B
        for u in range(max(P1B // 2, 1)):
            ch = (b0 + 2) // 2 + u

            @pl.when(ch < 8)
            def _():
                wait_rows(xbuf, ch * 256, 256, SEM_X + ch)
        wait_wgroup(i, i * JP1, JP1)
        for u in range(P1B):
            b = b0 + u
            bn = jnp.minimum(b + 1, NBLK - 1)
            weave(z2_tiles(b, u), ln_x(bn, (u + 1) % P1B))
            weave(z1_tiles(b, u), z2_post(b, u))
        for jj in range(JP1):
            relayout(i * JP1 + jj, wa, 0)
        return c
    lax.fori_loop(0, N1, ph1, 0)

    cp_wout.wait()

    def g_unit(g0, nrows, j):
        gh = pl.multiple_of(g0 // 2, 8)
        g = _dot(_bf(wsp[pl.ds(gh, nrows // 2), :]), _bf(z2[:, j * 128:(j + 1) * 128]))
        g = g + bcol[pl.ds(g0, nrows), :]
        u = (_gelu(z1[pl.ds(g0, nrows), j * 128:(j + 1) * 128]) * g).astype(BF16)
        ubuf[0:nrows // 2, j * 128:(j + 1) * 128] = _u32(u)

    def r_unit(b):
        h0 = pl.multiple_of(b * (SUB // 2), SUB // 2)
        lhs = jnp.concatenate([z2rt[k] for k in range(NBLK)], axis=1)
        gt = _dot_nt(_bf(lhs), _bf(wsp[pl.ds(h0, SUB // 2), :]))
        ut = _gelu(z1rt[b]) * (gt + brow[pl.ds(b, 1), :])
        urem[pl.ds(h0, SUB // 2), :] = _u32(jnp.transpose(ut).astype(BF16))

    def m_unit(g0, nrows, c):
        gh = pl.multiple_of(g0 // 2, 8)
        u = jnp.concatenate([ubuf[0:nrows // 2, :], urem[pl.ds(gh, nrows // 2), :]], axis=1)
        gm = _dot(_bf(u), _bf(wout[:, c * 128:(c + 1) * 128]))
        gate[pl.ds(g0, nrows), c * 128:(c + 1) * 128] = gm * jax.nn.sigmoid(gm)

    def ph2(m, c):
        wait_rows(wsp, m * WSPR, WSPR, SEM_WSP + m)
        j0 = N1 * JP1 + m * JP2
        wait_wgroup(N1 + m, j0, JP2)
        nr = P2B * SUB
        g0 = pl.multiple_of(m * nr, nr)
        rb = [m * 2 * P2B + u for u in range(2 * P2B)]
        hq0 = [m * (H // N2) + u for u in range(H // N2)]

        def q0_unit():
            if hq0:
                h = hq0.pop(0)
                qs[h] = _dot(xn[0:16, :].astype(BF16), _bf(wa[h]))[0:8]
        for j in range(NFT):
            g_unit(g0, nr, j)
            q0_unit()
            if j < len(rb):
                r_unit(rb[j])
        for cc in range(5):
            q0_unit()
            m_unit(g0, nr, cc)
        assert not hq0
        for jj in range(JP2):
            relayout(j0 + jj, wb, NA // 2)
        return c
    lax.fori_loop(0, N2, ph2, 0)
    cp_wo.wait()
    cp_mem0.wait()

    scheds = []
    for part in SCHED.split(';'):
        sched = {}
        for item in part.split(','):
            k, v = item.split(':')
            sched[k] = [v[n:n + 2] for n in range(0, len(v), 2)]
        scheds.append(sched)

    for sched in scheds:
        for us in sched.values():
            for u in us:
                if u[0] == 'n':
                    g_unit(R0, GR, int(u[1]))

    def pair(i, mem, sched, g0, g0n):
        zero = lax.shift_right_logical(i, 8)
        ok = _mask()
        r0 = pl.multiple_of(i * 64, 64)

        def run_step(hq, hh, first):
            o_ref = oa if first else ob
            name = 'A' if first else 'B'
            st = {}
            dep = {}
            acc = [None, 0]

            def wo_chunk(h0, h1):
                part = _dot(o_ref[:, h0 * 128:h1 * 128].astype(BF16), _bf(wo[h0 * 64:h1 * 64, :]))
                acc[0] = part if acc[0] is None else acc[0] + part
                acc[1] = h1

            def fillers(t):
                for u in sched.get('%s%d' % (name, t), []):
                    n = int(u[1])
                    if u[0] == 'g':
                        g_unit(g0, GR, n)
                    elif u[0] == 'n':
                        g_unit(g0n, GR, n)
                    elif u[0] == 'm':
                        m_unit(g0, GR, n)
                    elif u[0] == 'w':
                        wo_chunk(acc[1], acc[1] + 4)
                    elif u[0] == 'v':
                        wo_chunk(acc[1], acc[1] + n)

            SK_S, SK_PV = (SKA_S, SKA_PV) if first else (SKB_S, SKB_PV)

            I32 = jnp.int32
            sm = {}
            vp = {}

            def bits(x):
                return pltpu.bitcast(x, I32)

            def st_s(h):
                q, k, v = st[h]
                s = jnp.where(ok, _dot_nt(q, k) * (scale * LOG2E), -1e9 * LOG2E)
                sm[h] = dict(s=s, mx=jnp.max(s, axis=-1, keepdims=True))

            def st_e(h):
                d = sm[h]
                d['e'] = jnp.exp2(d['s'] - d['mx'])
                d['l'] = jnp.sum(d['e'], axis=-1, keepdims=True)

            base = 8 if first else 24
            shifts = list(range(-7, 9))

            def st_vr(h):
                q8 = (qs[h] if first else qv.pop(h)) * (scale * LOG2E)
                row = lax.broadcasted_iota(jnp.int32, (8, 1), 0)
                ss = []
                for d in shifts:
                    sj = jnp.sum(q8 * kvf[h, pl.ds(2 * (base + d), 8, stride=2), :], axis=-1, keepdims=True)
                    if d < 0:
                        sj = jnp.where(row >= -d, sj, -jnp.inf)
                    ss.append(sj)
                vp[h] = dict(ss=ss, mx=_tree(jnp.maximum, ss))

            def st_ve(h):
                dd = vp[h]
                es = [jnp.exp2(sj - dd['mx']) for sj in dd['ss']]
                l = _tree(jnp.add, es)
                o = _tree(jnp.add, [e * kvf[h, pl.ds(2 * (base + d) + 1, 8, stride=2), :] for e, d in zip(es, shifts)])
                r = pl.reciprocal(l, approx=True)
                r = r * (2.0 - l * r)
                o = o * r
                dd['o'] = o
                ro = 32 if first else 40
                ob[ro:ro + 8, h * 128:(h + 1) * 128] = o

            def put_kv(h, pos, rows):
                kvf[h, pl.ds(2 * pos, 8, stride=2), :] = rows[:, 0:128]
                kvf[h, pl.ds(2 * pos + 1, 8, stride=2), :] = rows[:, 128:256]

            def st_n(h):
                d = sm.pop(h)
                l = d['l']
                r = pl.reciprocal(l, approx=True)
                r = r * (2.0 - l * r)
                p = d['e'] * r
                toks32, toks8 = [], []
                if h + 2 < H:
                    toks32.append(sm[h + 2]['s'] - sm[h + 2]['mx'])
                if 0 <= h + 2 + DV < H:
                    toks8.append(jnp.broadcast_to(vp[h + 2 + DV]['mx'], (8, 40)))
                if h + 1 < H:
                    toks32.append(jnp.broadcast_to(sm[h + 1]['l'], (32, 40)))
                if 0 <= h + 1 + DV - DE < H:
                    toks8.append(vp[h + 1 + DV - DE]['o'][:, 0:40])
                if TOKREV:
                    toks32.reverse()
                    toks8.reverse()
                if toks32 and (TOKA if first else TOKB) & 1:
                    p = pltpu.bitcast((_tree(jnp.bitwise_or, [bits(x) for x in toks32]) & zero) | bits(p), F32)
                if toks8 and (TOKA if first else TOKB) & 2:
                    p0 = pltpu.bitcast((_tree(jnp.bitwise_or, [bits(x) for x in toks8]) & zero) | bits(p[0:8]), F32)
                    p = jnp.concatenate([p0, p[8:32]], axis=0)
                st[h] = (p.astype(BF16), st[h][2])

            def do_pv(h):
                p, v = st.pop(h)
                o_ref[0:32, h * 128:(h + 1) * 128] = _dot(p, v)

            qv = {}
            for t in range(H + SK_PV + 1):
                if t < H:
                    h = t
                    qf = _dot(hq, _bf(wslab(h)))
                    q = qf[0:32].astype(BF16)
                    kv = _dot(hh, _bf(jnp.concatenate([wslab(H + h), wslab(2 * H + h)], axis=1)))
                    if first:
                        put_kv(h, 8, kv[0:8])
                        put_kv(h, 16, kv[32:40])
                        put_kv(h, 32, kv[40:48])
                        k = kv[0:40, 0:128].astype(BF16)
                        v = kv[0:40, 128:256].astype(BF16)
                    else:
                        qv[h] = qf[32:40]
                        qs[h] = qf[40:48]
                        put_kv(h, 24, kv[0:8])
                        k = jnp.concatenate([kv[:, 0:128], kvf[h, pl.ds(64, 8, stride=2), :]], axis=0).astype(BF16)
                        v = jnp.concatenate([kv[:, 128:256], kvf[h, pl.ds(65, 8, stride=2), :]], axis=0).astype(BF16)
                    st[h] = (q, k, v)
                fillers(t)
                if 0 <= t - SK_PV < H:
                    do_pv(t - SK_PV)
                if 0 <= t - SK_S < H:
                    st_s(t - SK_S)
                if 0 <= t - SK_S + DV < H:
                    st_vr(t - SK_S + DV)
                if 0 <= t - SK_S - 1 < H:
                    st_e(t - SK_S - 1)
                if 0 <= t - SK_S - 1 + DV - DE < H:
                    st_ve(t - SK_S - 1 + DV - DE)
                if 0 <= t - SK_S - 2 < H:
                    st_n(t - SK_S - 2)
            wo_chunk(acc[1], H)
            res = acc[0]
            fillers(99)
            return res

        xt = xn[pl.ds(r0, 64), :]
        ha = jnp.concatenate([mem, xt[8:32], xt[0:8], xt[32:40]], axis=0).astype(BF16)
        sa = run_step(ha[0:32], ha, True)
        mem = sa[0:8]
        hb = jnp.concatenate([mem, xt[40:64]], axis=0).astype(BF16)
        rn = pl.multiple_of(jnp.minimum(r0 + 64, S - 8), 8)
        hx = jnp.concatenate([xt[32:40], xn[pl.ds(rn, 8), :]], axis=0).astype(BF16)
        sb = run_step(jnp.concatenate([hb, hx], axis=0), hb, False)
        mem = sb[0:8]
        sall = jnp.concatenate([sb[32:40], sa[8:32], sb[40:48], sb[8:32]], axis=0)
        xr = _bf(xbuf[pl.ds(pl.multiple_of(i * 32, 32), 32), :]).astype(F32)
        obuf[pl.ds(r0, 64), :] = (xr + sall * gate[pl.ds(r0, 64), :]).astype(BF16)
        return mem

    def body(ii, mem):
        g0 = pl.multiple_of(R0 + ii * GR, 16)
        g0n = pl.multiple_of(R0 + jnp.minimum(ii + 1, NBODY - 1) * GR, 16)
        for u in range(UNR):
            mem = pair(ii * UNR + u, mem, scheds[u], g0, g0n)
        r0 = pl.multiple_of(ii * (64 * UNR), 64 * UNR)
        pltpu.make_async_copy(obuf.at[pl.ds(r0, 64 * UNR), :], out_hbm.at[pl.ds(r0, 64 * UNR), :], osem).start()
        return mem

    lax.fori_loop(0, NBODY, body, mem0_ref[...].astype(F32))
    pltpu.make_async_copy(obuf, out_hbm, osem).wait()


@functools.partial(jax.jit, static_argnames=("A_seg_len",))
def pallas_recurrent_scan__memory_aug_recurrent_mem_tr__mixer_gmlp__prompt_kernel(A_x, A_mem0, A_Wq, A_Wk, A_Wv, A_Wo, A_seg_len, B_x, B_w_in, B_w_sp, B_b_sp, B_w_out):
    any_spec = pl.BlockSpec(memory_space=pl.ANY)
    vmem_spec = pl.BlockSpec(memory_space=pltpu.VMEM)
    out = pl.pallas_call(
        _kernel,
        out_shape=jax.ShapeDtypeStruct((S, D), BF16),
        in_specs=[any_spec] * 10,
        out_specs=any_spec,
        scratch_shapes=[
            pltpu.VMEM((S // 2, D), U32),
            pltpu.VMEM((S, D), F32),
            pltpu.VMEM((4, SUB // 2, D), U32),
            pltpu.VMEM((NJ, 2, D // 2, DH), U32),
            pltpu.VMEM((NA, D // 2, DH), U32),
            pltpu.VMEM((3 * H - NA, D // 2, DH), U32),
            pltpu.VMEM((H * DH // 2, D), U32),
            pltpu.VMEM((FH, D), U32),
            pltpu.VMEM((S // 2, S), U32),
            pltpu.VMEM((FH // 2, D), U32),
            pltpu.VMEM((S, FF), F32),
            pltpu.VMEM((NBLK, FR, SUB), F32),
            pltpu.VMEM((S // 2, FF), U32),
            pltpu.VMEM((NBLK, FR // 2, SUB), U32),
            pltpu.VMEM((4, SUB, FH), F32),
            pltpu.VMEM((S, 128), F32),
            pltpu.VMEM((16, 128), F32),
            pltpu.VMEM((S, D), F32),
            pltpu.VMEM((P2B * SUB // 2, FF), U32),
            pltpu.VMEM((S // 2, FR), U32),
            pltpu.VMEM((H, 80, DH), F32),
            pltpu.VMEM((H, 8, DH), F32),
            pltpu.VMEM((32, H * DH), F32),
            pltpu.VMEM((48, H * DH), F32),
            pltpu.VMEM((S, D), BF16),
            pltpu.VMEM((M, D), BF16),
            pltpu.VMEM((16, 128), BF16),
            pltpu.SemaphoreType.DMA((NSEM,)),
            pltpu.SemaphoreType.DMA,
        ],
        compiler_params=pltpu.CompilerParams(vmem_limit_bytes=110 * 1024 * 1024),
    )(A_x.reshape(S, D), A_mem0.reshape(M, D), A_Wq.reshape(D // 2, 2, H, DH), A_Wk.reshape(D // 2, 2, H, DH),
      A_Wv.reshape(D // 2, 2, H, DH), A_Wo.reshape(H * DH, D),
      B_w_in.T, B_w_sp, B_b_sp.reshape(16, 128), B_w_out)
    return out.reshape(1, S, D)
```

```python
import functools

import jax
import jax.numpy as jnp
from jax import lax
import jax.experimental.pallas as pl
import jax.experimental.pallas.tpu as pltpu

F32 = jnp.float32
BF16 = jnp.bfloat16
U32 = jnp.uint32
I32 = jnp.int32

S, D, H, DH, M, SEG = 2048, 640, 32, 128, 8, 32
FH = 864
FF = 768
FR = FH - FF
NFT = FF // 128
EPS = 1e-5
LOG2E = 1.4426950408889634

NPAIR = S // (2 * SEG)
UNR = 2
NBODY = NPAIR // UNR
SUB = 128
NBLK = S // SUB
R0 = 1024
GR = (S - R0) // NBODY
P1B = 2
P2B = 2
N1 = (NBLK - 4) // P1B
N2 = (R0 // SUB) // P2B
NJ = 3 * H // 2
JP1 = 4
JP2 = (NJ - N1 * JP1) // N2
NA = 2 * N1 * JP1
WSPR = S // N2
assert N1 * JP1 + N2 * JP2 == NJ and NA >= H

SK_S, SKA_PV, SKB_PV, VLAG = 2, 5, 7, 3
SCHED = (
    {'A32': 'g1', 'A33': 'w', 'A34': 'w', 'A35': 'w', 'A36': 'w', 'Aend': 'g2',
     'B32': 'g3', 'B33': 'w', 'B34': 'w', 'B35': 'w', 'B36': 'w', 'Bend': 'g4'},
    {'A32': 'g5', 'A33': 'w', 'A34': 'w', 'A35': 'w', 'A36': 'w', 'Aend': 'm0 m1',
     'B32': 'm2 m3', 'B33': 'm4', 'B34': 'w', 'B35': 'w', 'B36': 'w', 'Bend': 'n0'},
)
NCH = 4
LN_PLAN = {
    0: [('x', 0, 0, 0)], 1: [('x', 1, 0, 1)], 2: [('x', 1, 1, 1)], 3: [('x', 1, 2, 1), ('x', 1, 3, 1)],
    4: [('x', 2, 0, 1)], 6: [('z', 0, 0, 0)],
    7: [('z', 1, 0, 0), ('z', 1, 1, 0), ('z', 1, 2, 0), ('z', 1, 3, 0)],
    8: [('z', 2, 0, 0), ('z', 2, 1, 0)], 9: [('z', 2, 2, 1), ('x', 2, 1, 1)],
    10: [('z', 2, 3, 1), ('x', 2, 2, 1)], 11: [('x', 2, 3, 1)],
}

SEM_X = 0
SEM_WIN = 8
SEM_W = 11
SEM_WOUT = SEM_W + N1 + N2
SEM_WSP = SEM_WOUT + 1
SEM_WO = SEM_WSP + N2
SEM_SMALL = SEM_WO + 1
NSEM = SEM_SMALL + 2


def _bf(x):
    return pltpu.bitcast(x, BF16)


def _u32(x):
    return pltpu.bitcast(x, U32)


def _bits(x):
    return pltpu.bitcast(x, I32)


def _dot(a, b):
    return jnp.dot(a, b, preferred_element_type=F32)


def _dot_nt(a, b):
    return lax.dot_general(a, b, (((1,), (1,)), ((), ())), preferred_element_type=F32)


def _gelu(x):
    c = 0.7978845608028654
    t = jnp.tanh(x * (c + (c * 0.044715) * (x * x)))
    hx = 0.5 * x
    return hx + hx * t


def _recip(l):
    r = pl.reciprocal(l, approx=True)
    return r * (2.0 - l * r)


def _tree(op, xs):
    xs = list(xs)
    while len(xs) > 1:
        xs = [op(xs[n], xs[n + 1]) if n + 1 < len(xs) else xs[n] for n in range(0, len(xs), 2)]
    return xs[0]


def _mask():
    qi = lax.broadcasted_iota(I32, (32, 40), 0)
    ki = lax.broadcasted_iota(I32, (32, 40), 1)
    return (qi < 8) | (ki < 8) | (ki >= 32) | (qi >= ki)


def _kernel(x_hbm, mem0_hbm, wq_hbm, wk_hbm, wv_hbm, wo_hbm, wint_hbm, wsp_hbm, bsp_hbm, wout_hbm,
            out_hbm,
            xbuf, xn, xnb, wraw, wa, wb, wo, wint, wsp, wout, z1, z1rt, z2, z2rt, ztmp, bcol, brow,
            gate, ubuf, urem, kvf, qs, oa, ob, obuf, mem0_ref, bsp_ref, sems, osem):
    qscale = DH ** -0.5 * LOG2E

    w32 = [w.bitcast(U32) for w in (wq_hbm, wk_hbm, wv_hbm)]
    x32 = x_hbm.bitcast(U32)
    wsp32 = wsp_hbm.bitcast(U32)
    wint32 = wint_hbm.bitcast(U32)

    def cp_rows(src, dst, r0, n, sem):
        return pltpu.make_async_copy(src.at[pl.ds(r0 // 2, n // 2)], dst.at[pl.ds(r0 // 2, n // 2)], sems.at[sem])

    def wait_rows(dst, r0, n, sem):
        d = dst.at[pl.ds(pl.multiple_of(r0 // 2, 8), n // 2)]
        pltpu.make_async_copy(d, d, sems.at[sem]).wait()

    def wgroup(k):
        j0, n = (k * JP1, JP1) if k < N1 else (N1 * JP1 + (k - N1) * JP2, JP2)
        return [pltpu.make_async_copy(w32[J // 16].at[:, p, J % 16, :], wraw.at[J, p], sems.at[SEM_W + k])
                for J in range(j0, j0 + n) for p in range(2)]

    def wait_wgroup(k, j0, n):
        wgrp = wraw.at[pl.ds(j0, n)]
        pltpu.make_async_copy(wgrp, wgrp, sems.at[SEM_W + k]).wait()

    cp_x = [cp_rows(x32, xbuf, j * 256, 256, SEM_X + j) for j in range(8)]
    cp_win = [cp_rows(wint32, wint, FH, 512, SEM_WIN), cp_rows(wint32, wint, FH + 512, FH - 512, SEM_WIN + 1),
              cp_rows(wint32, wint, FF, FR, SEM_WIN + 1), cp_rows(wint32, wint, 0, FF, SEM_WIN + 2)]
    cp_wout = pltpu.make_async_copy(wout_hbm.bitcast(U32), wout, sems.at[SEM_WOUT])
    cp_wsp = [cp_rows(wsp32, wsp, m * WSPR, WSPR, SEM_WSP + m) for m in range(N2)]
    cp_wo = pltpu.make_async_copy(wo_hbm.bitcast(U32), wo, sems.at[SEM_WO])
    cp_bsp = pltpu.make_async_copy(bsp_hbm, bsp_ref, sems.at[SEM_SMALL])
    cp_mem0 = pltpu.make_async_copy(mem0_hbm, mem0_ref, sems.at[SEM_SMALL + 1])

    dma = [cp_bsp, cp_x[0], cp_win[0], cp_x[1], cp_mem0, cp_win[1], cp_win[2], cp_win[3], cp_x[2]]
    for k in range(N1):
        dma += cp_x[3 + k:4 + k] + wgroup(k)
    dma += [cp_wout]
    for m in range(N2):
        dma += [cp_wsp[m]] + wgroup(N1 + m)
        if m == N2 - 2:
            dma.append(cp_wo)
    nb = -(-len(dma) // 4)
    batches = [dma[b * nb:(b + 1) * nb] for b in range(4)]

    def start_all(cps):
        for c in cps:
            c.start()

    start_all(batches[0])

    cp_bsp.wait()
    bsp = bsp_ref[...].astype(F32)
    brow[...] = bsp
    kvf[:, 0:16, :] = jnp.zeros((H, 16, DH), F32)
    for c in range(16):
        bcol[c * 128:(c + 1) * 128, :] = jnp.transpose(jnp.broadcast_to(bsp[c:c + 1, :], (128, 128)))

    def ln_passes(ld, fin):
        st = {}

        def p0():
            st['m'] = jnp.mean(ld(), axis=-1, keepdims=True)

        def p1():
            c = ld() - st['m']
            st['r'] = lax.rsqrt(jnp.mean(c * c, axis=-1, keepdims=True) + EPS)

        def p2():
            fin((ld() - st['m']) * st['r'])
        return [p0, p1, p2]

    def ln_x(b, s):
        def fin(v):
            xn[b * SUB:(b + 1) * SUB, :] = v
            xnb[s] = _u32(v.astype(BF16))
        return ln_passes(lambda: _bf(xbuf[b * (SUB // 2):(b + 1) * (SUB // 2), :]).astype(F32), fin)

    def z2_post(b, s):
        def fin(v):
            z2[b * (SUB // 2):(b + 1) * (SUB // 2), :] = _u32(v[:, 0:FF].astype(BF16))
            z2rt[b] = _u32(jnp.transpose(v[:, FF:FH]).astype(BF16))
        return ln_passes(lambda: ztmp[s], fin)

    def z2_tiles(b, s):
        def tile(j):
            lo = (FH + j * 128) // 2
            t = _gelu(_dot_nt(_bf(xnb[s]), _bf(wint[lo:lo + 64, :])))
            ztmp[s, :, j * 128:(j + 1) * 128] = t
            return t[0:8]

        def rem():
            wr = jnp.concatenate([wint[FF // 2:FH // 2, :], wint[(FH + FF) // 2:FH, :]], axis=0)
            zr = _dot_nt(_bf(wr), _bf(xnb[s]))
            z1rt[b] = zr[0:FR]
            ztmp[s, :, FF:FH] = jnp.transpose(_gelu(zr[FR:2 * FR]))
            return zr[0:8]
        return ([functools.partial(tile, j) for j in range(4)] + [rem]
                + [functools.partial(tile, j) for j in range(4, NFT)])

    def z1_tiles(b, s):
        r0 = pl.multiple_of(b * SUB, SUB)

        def tile(j):
            t = _dot_nt(_bf(xnb[s]), _bf(wint[j * 64:(j + 1) * 64, :]))
            z1[pl.ds(r0, SUB), j * 128:(j + 1) * 128] = t
            return t[0:8]
        return [functools.partial(tile, j) for j in range(NFT)]

    def weave(tiles, *passes):
        for n, t in enumerate(tiles):
            t()
            if n % 2 == 0 and n // 2 < 3:
                for p in passes:
                    p[n // 2]()

    def relayout(J, dst, j0):
        for r in range(0, D // 2, 80):
            ev = wraw[J, 0, r:r + 80, :]
            od = wraw[J, 1, r:r + 80, :]
            dst[2 * (J - j0), r:r + 80, :] = (ev & jnp.uint32(0xFFFF)) | (od << 16)
            dst[2 * (J - j0) + 1, r:r + 80, :] = (ev >> 16) | (od & jnp.uint32(0xFFFF0000))

    def wslab(n):
        return wa[n] if n < NA else wb[n - NA]

    cp_x[0].wait()
    for p in ln_x(0, 0) + ln_x(1, 1):
        p()
    cp_win[0].wait()
    t0, t1 = z2_tiles(0, 0), z2_tiles(1, 1)
    weave(t0[0:4] + t1[0:4])
    start_all(batches[1])
    cp_x[1].wait()
    cp_win[1].wait()
    cp_win[2].wait()
    weave(t0[4:] + t1[4:], ln_x(2, 2), ln_x(3, 3))
    weave(z2_tiles(2, 2), z2_post(0, 0))
    weave(z2_tiles(3, 3), z2_post(1, 1))
    cp_win[3].wait()
    cp_x[2].wait()
    weave(z1_tiles(0, 0), z2_post(2, 2))
    weave(z1_tiles(1, 1), z2_post(3, 3))
    weave(z1_tiles(2, 2), ln_x(4, 0))
    weave(z1_tiles(3, 3))

    def ln_chunked(ld, fin, zero, width):
        n = SUB // NCH
        st = {}

        def mean_of(c, tok):
            m = st['m'][c]
            if tok is None:
                return m
            t = jnp.concatenate([_bits(tok) & zero] * (n // 8), axis=0)
            mb = pltpu.bitcast(_bits(jnp.broadcast_to(m, (n, 128))) | t, F32)
            return jnp.concatenate([mb] * (-(-width // 128)), axis=1)[:, 0:width]

        def run(stage, c, tok):
            if stage == 0:
                st['m'] = [jnp.mean(ld(q * n, n), axis=-1, keepdims=True) for q in range(NCH)]
                st['r'] = [None] * NCH
            elif stage == 1:
                m = mean_of(c, tok)
                d = ld(c * n, n) - m
                st['r'][c] = lax.rsqrt(jnp.mean(d * d, axis=-1, keepdims=True) + EPS)
            else:
                m = mean_of(c, tok)
                fin(c * n, n, (ld(c * n, n) - m) * st['r'][c])
        return run

    def ph1(i, carry):
        @pl.when(i == N1 // 3)
        def _():
            start_all(batches[2])

        @pl.when(i == (2 * N1) // 3)
        def _():
            start_all(batches[3])
        b0 = 4 + i * P1B
        ch = (b0 + 2) // 2

        @pl.when(ch < 8)
        def _():
            wait_rows(xbuf, ch * 256, 256, SEM_X + ch)
        wait_wgroup(i, i * JP1, JP1)
        zero = lax.shift_right_logical(i, 8)
        for u in range(P1B):
            b = b0 + u
            bn = jnp.minimum(b + 1, NBLK - 1)
            sn = (u + 1) % P1B
            vrem = {}

            def ldx(r, n, bn=bn):
                return _bf(xbuf[pl.ds(pl.multiple_of(bn * (SUB // 2) + r // 2, 8), n // 2), :]).astype(F32)

            def finx(r, n, v, bn=bn, sn=sn):
                xn[pl.ds(pl.multiple_of(bn * SUB + r, 16), n), :] = v
                xnb[sn, r // 2:(r + n) // 2, :] = _u32(v.astype(BF16))

            def ldz(r, n, u=u):
                return ztmp[u, r:r + n, :]

            def finz(r, n, v, b=b, vrem=vrem):
                z2[pl.ds(pl.multiple_of(b * (SUB // 2) + r // 2, 8), n // 2), :] = _u32(v[:, 0:FF].astype(BF16))
                vrem[r] = v[:, FF:FH]
                if r + n == SUB:
                    vr = jnp.concatenate([vrem[k] for k in sorted(vrem)], axis=0)
                    z2rt[b] = _u32(jnp.transpose(vr).astype(BF16))
            lns = {'x': ln_chunked(ldx, finx, zero, D), 'z': ln_chunked(ldz, finz, zero, FH)}
            for n, t in enumerate(z2_tiles(b, u) + z1_tiles(b, u)):
                tok = t()
                for which, stage, c, anchored in LN_PLAN.get(n, []):
                    lns[which](stage, c, tok if anchored else None)
        for jj in range(JP1):
            relayout(i * JP1 + jj, wa, 0)
        return carry
    lax.fori_loop(0, N1, ph1, 0)

    cp_wout.wait()

    def g_unit(g0, nrows, j):
        gh = pl.multiple_of(g0 // 2, 8)
        g = _dot(_bf(wsp[pl.ds(gh, nrows // 2), :]), _bf(z2[:, j * 128:(j + 1) * 128]))
        g = g + bcol[pl.ds(g0, nrows), :]
        u = (_gelu(z1[pl.ds(g0, nrows), j * 128:(j + 1) * 128]) * g).astype(BF16)
        ubuf[0:nrows // 2, j * 128:(j + 1) * 128] = _u32(u)

    def r_unit(b):
        h0 = pl.multiple_of(b * (SUB // 2), SUB // 2)
        lhs = jnp.concatenate([z2rt[k] for k in range(NBLK)], axis=1)
        gt = _dot_nt(_bf(lhs), _bf(wsp[pl.ds(h0, SUB // 2), :]))
        ut = _gelu(z1rt[b]) * (gt + brow[pl.ds(b, 1), :])
        urem[pl.ds(h0, SUB // 2), :] = _u32(jnp.transpose(ut).astype(BF16))

    def m_unit(g0, nrows, c):
        gh = pl.multiple_of(g0 // 2, 8)
        u = jnp.concatenate([ubuf[0:nrows // 2, :], urem[pl.ds(gh, nrows // 2), :]], axis=1)
        gm = _dot(_bf(u), _bf(wout[:, c * 128:(c + 1) * 128]))
        gate[pl.ds(g0, nrows), c * 128:(c + 1) * 128] = gm * jax.nn.sigmoid(gm)

    def ph2(m, carry):
        wait_rows(wsp, m * WSPR, WSPR, SEM_WSP + m)
        j0 = N1 * JP1 + m * JP2
        wait_wgroup(N1 + m, j0, JP2)
        nr = P2B * SUB
        g0 = pl.multiple_of(m * nr, nr)
        rb = [m * 2 * P2B + u for u in range(2 * P2B)]
        hq0 = [m * (H // N2) + u for u in range(H // N2)]

        def q0_unit():
            if hq0:
                h = hq0.pop(0)
                qs[h] = _dot(xn[0:16, :].astype(BF16), _bf(wa[h]))[0:8]
        for j in range(NFT):
            g_unit(g0, nr, j)
            q0_unit()
            if j < len(rb):
                r_unit(rb[j])
        for cc in range(5):
            q0_unit()
            m_unit(g0, nr, cc)
        assert not hq0 and len(rb) <= NFT
        for jj in range(JP2):
            relayout(j0 + jj, wb, NA // 2)
        return carry
    lax.fori_loop(0, N2, ph2, 0)
    cp_wo.wait()
    cp_mem0.wait()
    g_unit(R0, GR, 0)

    def pair(i, mem, sched, g0, g0n):
        zero = lax.shift_right_logical(i, 8)
        ok = _mask()
        r0 = pl.multiple_of(i * 64, 64)

        def run_step(hq, hh, first):
            o_ref = oa if first else ob
            sk_pv = SKA_PV if first else SKB_PV
            st, sm, vp, qv = {}, {}, {}, {}
            acc = [None, 0]

            def wo_chunk(h1):
                h0 = acc[1]
                part = _dot(o_ref[:, h0 * 128:h1 * 128].astype(BF16), _bf(wo[h0 * 64:h1 * 64, :]))
                acc[0] = part if acc[0] is None else acc[0] + part
                acc[1] = h1

            def fillers(slot):
                for u in sched.get(('A' if first else 'B') + str(slot), '').split():
                    if u[0] == 'g':
                        g_unit(g0, GR, int(u[1]))
                    elif u[0] == 'n':
                        g_unit(g0n, GR, int(u[1]))
                    elif u[0] == 'm':
                        m_unit(g0, GR, int(u[1]))
                    else:
                        wo_chunk(acc[1] + 4)

            def scores(h):
                q, k, _ = st[h]
                s = jnp.where(ok, _dot_nt(q, k) * qscale, -1e9 * LOG2E)
                sm[h] = dict(s=s, mx=jnp.max(s, axis=-1, keepdims=True))

            def exps(h):
                d = sm[h]
                d['e'] = jnp.exp2(d['s'] - d['mx'])
                d['l'] = jnp.sum(d['e'], axis=-1, keepdims=True)

            base = 8 if first else 24
            shifts = list(range(-7, 9))

            def vpu_scores(h):
                q8 = (qs[h] if first else qv.pop(h)) * qscale
                row = lax.broadcasted_iota(I32, (8, 1), 0)
                ss = []
                for d in shifts:
                    sj = jnp.sum(q8 * kvf[h, pl.ds(2 * (base + d), 8, stride=2), :], axis=-1, keepdims=True)
                    if d < 0:
                        sj = jnp.where(row >= -d, sj, -jnp.inf)
                    ss.append(sj)
                vp[h] = dict(ss=ss, mx=_tree(jnp.maximum, ss))

            def vpu_out(h):
                dd = vp[h]
                es = [jnp.exp2(sj - dd['mx']) for sj in dd['ss']]
                l = _tree(jnp.add, es)
                o = _tree(jnp.add, [e * kvf[h, pl.ds(2 * (base + d) + 1, 8, stride=2), :]
                                    for e, d in zip(es, shifts)])
                o = o * _recip(l)
                dd['o'] = o
                ro = 32 if first else 40
                ob[ro:ro + 8, h * 128:(h + 1) * 128] = o

            def put_kv(h, pos, rows):
                kvf[h, pl.ds(2 * pos, 8, stride=2), :] = rows[:, 0:128]
                kvf[h, pl.ds(2 * pos + 1, 8, stride=2), :] = rows[:, 128:256]

            def normalize(h):
                d = sm.pop(h)
                p = d['e'] * _recip(d['l'])
                toks32, toks8 = [], []
                if h + 2 < H:
                    toks32.append(sm[h + 2]['s'] - sm[h + 2]['mx'])
                if 0 <= h + 2 - VLAG < H:
                    toks8.append(jnp.broadcast_to(vp[h + 2 - VLAG]['mx'], (8, 40)))
                if h + 1 < H:
                    toks32.append(jnp.broadcast_to(sm[h + 1]['l'], (32, 40)))
                if 0 <= h + 1 - VLAG < H:
                    toks8.append(vp[h + 1 - VLAG]['o'][:, 0:40])
                if toks32 and not first:
                    p = pltpu.bitcast((_tree(jnp.bitwise_or, [_bits(x) for x in toks32]) & zero) | _bits(p), F32)
                if toks8:
                    p0 = pltpu.bitcast((_tree(jnp.bitwise_or, [_bits(x) for x in toks8]) & zero)
                                       | _bits(p[0:8]), F32)
                    p = jnp.concatenate([p0, p[8:32]], axis=0)
                st[h] = (p.astype(BF16), st[h][2])

            def pv(h):
                p, v = st.pop(h)
                o_ref[0:32, h * 128:(h + 1) * 128] = _dot(p, v)

            assert SK_S + 1 + VLAG <= sk_pv + 1
            for t in range(H + sk_pv + 1):
                if t < H:
                    h = t
                    qf = _dot(hq, _bf(wslab(h)))
                    q = qf[0:32].astype(BF16)
                    kv = _dot(hh, _bf(jnp.concatenate([wslab(H + h), wslab(2 * H + h)], axis=1)))
                    if first:
                        put_kv(h, 8, kv[0:8])
                        put_kv(h, 16, kv[32:40])
                        put_kv(h, 32, kv[40:48])
                        k = kv[0:40, 0:128].astype(BF16)
                        v = kv[0:40, 128:256].astype(BF16)
                    else:
                        qv[h] = qf[32:40]
                        qs[h] = qf[40:48]
                        put_kv(h, 24, kv[0:8])
                        k = jnp.concatenate([kv[:, 0:128], kvf[h, pl.ds(64, 8, stride=2), :]], axis=0).astype(BF16)
                        v = jnp.concatenate([kv[:, 128:256], kvf[h, pl.ds(65, 8, stride=2), :]], axis=0).astype(BF16)
                    st[h] = (q, k, v)
                fillers(t)
                for lag, stage in ((sk_pv, pv), (SK_S, scores), (SK_S + VLAG, vpu_scores), (SK_S + 1, exps),
                                   (SK_S + 1 + VLAG, vpu_out), (SK_S + 2, normalize)):
                    if 0 <= t - lag < H:
                        stage(t - lag)
            wo_chunk(H)
            res = acc[0]
            fillers('end')
            return res

        xt = xn[pl.ds(r0, 64), :]
        ha = jnp.concatenate([mem, xt[8:32], xt[0:8], xt[32:40]], axis=0).astype(BF16)
        sa = run_step(ha[0:32], ha, True)
        mem = sa[0:8]
        hb = jnp.concatenate([mem, xt[40:64]], axis=0).astype(BF16)
        rn = pl.multiple_of(jnp.minimum(r0 + 64, S - 8), 8)
        hx = jnp.concatenate([xt[32:40], xn[pl.ds(rn, 8), :]], axis=0).astype(BF16)
        sb = run_step(jnp.concatenate([hb, hx], axis=0), hb, False)
        mem = sb[0:8]
        sall = jnp.concatenate([sb[32:40], sa[8:32], sb[40:48], sb[8:32]], axis=0)
        xr = _bf(xbuf[pl.ds(pl.multiple_of(i * 32, 32), 32), :]).astype(F32)
        obuf[pl.ds(r0, 64), :] = (xr + sall * gate[pl.ds(r0, 64), :]).astype(BF16)
        return mem

    def body(ii, mem):
        g0 = pl.multiple_of(R0 + ii * GR, 16)
        g0n = pl.multiple_of(R0 + jnp.minimum(ii + 1, NBODY - 1) * GR, 16)
        for u in range(UNR):
            mem = pair(ii * UNR + u, mem, SCHED[u], g0, g0n)
        r0 = pl.multiple_of(ii * (64 * UNR), 64 * UNR)
        pltpu.make_async_copy(obuf.at[pl.ds(r0, 64 * UNR), :], out_hbm.at[pl.ds(r0, 64 * UNR), :], osem).start()
        return mem

    lax.fori_loop(0, NBODY, body, mem0_ref[...].astype(F32))
    pltpu.make_async_copy(obuf, out_hbm, osem).wait()


@functools.partial(jax.jit, static_argnames=("A_seg_len",))
def pallas_recurrent_scan__memory_aug_recurrent_mem_tr__mixer_gmlp__prompt_kernel(A_x, A_mem0, A_Wq, A_Wk, A_Wv, A_Wo, A_seg_len, B_x, B_w_in, B_w_sp, B_b_sp, B_w_out):
    assert A_seg_len == SEG and A_x.shape == (1, S, D) and A_mem0.shape == (1, M, D)
    any_spec = pl.BlockSpec(memory_space=pl.ANY)
    out = pl.pallas_call(
        _kernel,
        out_shape=jax.ShapeDtypeStruct((S, D), BF16),
        in_specs=[any_spec] * 10,
        out_specs=any_spec,
        scratch_shapes=[
            pltpu.VMEM((S // 2, D), U32),
            pltpu.VMEM((S, D), F32),
            pltpu.VMEM((4, SUB // 2, D), U32),
            pltpu.VMEM((NJ, 2, D // 2, DH), U32),
            pltpu.VMEM((NA, D // 2, DH), U32),
            pltpu.VMEM((3 * H - NA, D // 2, DH), U32),
            pltpu.VMEM((H * DH // 2, D), U32),
            pltpu.VMEM((FH, D), U32),
            pltpu.VMEM((S // 2, S), U32),
            pltpu.VMEM((FH // 2, D), U32),
            pltpu.VMEM((S, FF), F32),
            pltpu.VMEM((NBLK, FR, SUB), F32),
            pltpu.VMEM((S // 2, FF), U32),
            pltpu.VMEM((NBLK, FR // 2, SUB), U32),
            pltpu.VMEM((4, SUB, FH), F32),
            pltpu.VMEM((S, 128), F32),
            pltpu.VMEM((16, 128), F32),
            pltpu.VMEM((S, D), F32),
            pltpu.VMEM((P2B * SUB // 2, FF), U32),
            pltpu.VMEM((S // 2, FR), U32),
            pltpu.VMEM((H, 88, DH), F32),
            pltpu.VMEM((H, 8, DH), F32),
            pltpu.VMEM((32, H * DH), F32),
            pltpu.VMEM((48, H * DH), F32),
            pltpu.VMEM((S, D), BF16),
            pltpu.VMEM((M, D), BF16),
            pltpu.VMEM((16, 128), BF16),
            pltpu.SemaphoreType.DMA((NSEM,)),
            pltpu.SemaphoreType.DMA,
        ],
        compiler_params=pltpu.CompilerParams(vmem_limit_bytes=110 * 1024 * 1024),
    )(A_x.reshape(S, D), A_mem0.reshape(M, D), A_Wq.reshape(D // 2, 2, H, DH), A_Wk.reshape(D // 2, 2, H, DH),
      A_Wv.reshape(D // 2, 2, H, DH), A_Wo.reshape(H * DH, D),
      B_w_in.T, B_w_sp, B_b_sp.reshape(16, 128), B_w_out)
    return out.reshape(1, S, D)
```

```python
import functools

import jax
import jax.numpy as jnp
from jax import lax
import jax.experimental.pallas as pl
import jax.experimental.pallas.tpu as pltpu

F32 = jnp.float32
BF16 = jnp.bfloat16
U32 = jnp.uint32
I32 = jnp.int32

S, D, H, DH, M, SEG = 2048, 640, 32, 128, 8, 32
FH = 864
FF = 768
FR = FH - FF
NFT = FF // 128
EPS = 1e-5
LOG2E = 1.4426950408889634

NPAIR = S // (2 * SEG)
UNR = 2
NBODY = NPAIR // UNR
SUB = 128
NBLK = S // SUB
R0 = 1024
GR = (S - R0) // NBODY
P1B = 2
P2B = 2
N1 = (NBLK - 4) // P1B
N2 = (R0 // SUB) // P2B
NJ = 3 * H // 2
JP1 = 4
JP2 = (NJ - N1 * JP1) // N2
NA = 2 * N1 * JP1
WSPR = S // N2
assert N1 * JP1 + N2 * JP2 == NJ and NA >= H

SK_S, SKA_PV, SKB_PV, VLAG = 2, 5, 7, 3
SCHED = (
    {'A32': 'g1', 'A33': 'w', 'A34': 'w', 'A35': 'w', 'A36': 'w', 'Aend': 'g2',
     'B32': 'g3', 'B33': 'w', 'B34': 'w', 'B35': 'w', 'B36': 'w', 'Bend': 'g4'},
    {'A32': 'g5', 'A33': 'w', 'A34': 'w', 'A35': 'w', 'A36': 'w', 'Aend': 'm0 m1',
     'B32': 'm2 m3', 'B33': 'm4', 'B34': 'w', 'B35': 'w', 'B36': 'w', 'Bend': 'n0'},
)
NCH = 4
LN_PLAN = {
    0: [('x', 0, 0, 0)], 1: [('x', 1, 0, 1)], 2: [('x', 1, 1, 1)], 3: [('x', 1, 2, 1), ('x', 1, 3, 1)],
    4: [('x', 2, 0, 1)], 6: [('z', 0, 0, 0)],
    7: [('z', 1, 0, 0), ('z', 1, 1, 0), ('z', 1, 2, 0), ('z', 1, 3, 0)],
    8: [('z', 2, 0, 0), ('z', 2, 1, 0)], 9: [('z', 2, 2, 1), ('x', 2, 1, 1)],
    10: [('z', 2, 3, 1), ('x', 2, 2, 1)], 11: [('x', 2, 3, 1)],
}

SEM_X = 0
SEM_WIN = 8
SEM_W = 11
SEM_WOUT = SEM_W + N1 + N2
SEM_WSP = SEM_WOUT + 1
SEM_WO = SEM_WSP + N2
SEM_SMALL = SEM_WO + 1
NSEM = SEM_SMALL + 2


def _bf(x):
    return pltpu.bitcast(x, BF16)


def _u32(x):
    return pltpu.bitcast(x, U32)


def _bits(x):
    return pltpu.bitcast(x, I32)


def _dot(a, b):
    return jnp.dot(a, b, preferred_element_type=F32)


def _dot_nt(a, b):
    return lax.dot_general(a, b, (((1,), (1,)), ((), ())), preferred_element_type=F32)


def _gelu(x):
    c = 0.7978845608028654
    t = jnp.tanh(x * (c + (c * 0.044715) * (x * x)))
    hx = 0.5 * x
    return hx + hx * t


def _recip(l):
    r = pl.reciprocal(l, approx=True)
    return r * (2.0 - l * r)


def _tree(op, xs):
    xs = list(xs)
    while len(xs) > 1:
        xs = [op(xs[n], xs[n + 1]) if n + 1 < len(xs) else xs[n] for n in range(0, len(xs), 2)]
    return xs[0]


def _mask():
    qi = lax.broadcasted_iota(I32, (32, 40), 0)
    ki = lax.broadcasted_iota(I32, (32, 40), 1)
    return (qi < 8) | (ki < 8) | (ki >= 32) | (qi >= ki)


def _kernel(x_hbm, mem0_hbm, wq_hbm, wk_hbm, wv_hbm, wo_hbm, wint_hbm, wsp_hbm, bsp_hbm, wout_hbm,
            out_hbm,
            xbuf, xn, xnb, wraw, wa, wb, wo, wint, wsp, wout, z1, z1rt, z2, z2rt, ztmp, bcol, brow,
            gate, ubuf, urem, kvf, qs, oa, ob, obuf, mem0_ref, bsp_ref, sems, osem):
    qscale = DH ** -0.5 * LOG2E

    w32 = [w.bitcast(U32) for w in (wq_hbm, wk_hbm, wv_hbm)]
    x32 = x_hbm.bitcast(U32)
    wsp32 = wsp_hbm.bitcast(U32)
    wint32 = wint_hbm.bitcast(U32)

    def cp_rows(src, dst, r0, n, sem):
        return pltpu.make_async_copy(src.at[pl.ds(r0 // 2, n // 2)], dst.at[pl.ds(r0 // 2, n // 2)], sems.at[sem])

    def wait_rows(dst, r0, n, sem):
        d = dst.at[pl.ds(pl.multiple_of(r0 // 2, 8), n // 2)]
        pltpu.make_async_copy(d, d, sems.at[sem]).wait()

    def wgroup(k):
        j0, n = (k * JP1, JP1) if k < N1 else (N1 * JP1 + (k - N1) * JP2, JP2)
        return [pltpu.make_async_copy(w32[J // 16].at[:, J % 16, :], wraw.at[J, pl.ds(0, D)], sems.at[SEM_W + k])
                for J in range(j0, j0 + n)]

    def wait_wgroup(k, j0, n):
        wgrp = wraw.at[pl.ds(j0, n), pl.ds(0, D)]
        pltpu.make_async_copy(wgrp, wgrp, sems.at[SEM_W + k]).wait()

    cp_x = [cp_rows(x32, xbuf, j * 256, 256, SEM_X + j) for j in range(8)]
    cp_win = [cp_rows(wint32, wint, FH, 512, SEM_WIN), cp_rows(wint32, wint, FH + 512, FH - 512, SEM_WIN + 1),
              cp_rows(wint32, wint, FF, FR, SEM_WIN + 1), cp_rows(wint32, wint, 0, FF, SEM_WIN + 2)]
    cp_wout = pltpu.make_async_copy(wout_hbm.bitcast(U32), wout, sems.at[SEM_WOUT])
    cp_wsp = [cp_rows(wsp32, wsp, m * WSPR, WSPR, SEM_WSP + m) for m in range(N2)]
    cp_wo = pltpu.make_async_copy(wo_hbm.bitcast(U32), wo, sems.at[SEM_WO])
    cp_bsp = pltpu.make_async_copy(bsp_hbm, bsp_ref, sems.at[SEM_SMALL])
    cp_mem0 = pltpu.make_async_copy(mem0_hbm, mem0_ref, sems.at[SEM_SMALL + 1])

    dma = [cp_bsp, cp_x[0], cp_win[0], cp_x[1], cp_mem0, cp_win[1], cp_win[2], cp_win[3], cp_x[2]]
    for k in range(N1):
        dma += cp_x[3 + k:4 + k] + wgroup(k)
    dma += [cp_wout]
    for m in range(N2):
        dma += [cp_wsp[m]] + wgroup(N1 + m)
        if m == N2 - 2:
            dma.append(cp_wo)
    batches = [dma[0:50], dma[50:]]

    def start_all(cps):
        for c in cps:
            c.start()

    start_all(batches[0])

    cp_bsp.wait()
    bsp = bsp_ref[...].astype(F32)
    brow[...] = bsp
    kvf[:, 0:16, :] = jnp.zeros((H, 16, DH), F32)
    for c in range(16):
        bcol[c * 128:(c + 1) * 128, :] = jnp.transpose(jnp.broadcast_to(bsp[c:c + 1, :], (128, 128)))

    def ln_passes(ld, fin):
        st = {}

        def p0():
            st['m'] = jnp.mean(ld(), axis=-1, keepdims=True)

        def p1():
            c = ld() - st['m']
            st['r'] = lax.rsqrt(jnp.mean(c * c, axis=-1, keepdims=True) + EPS)

        def p2():
            fin((ld() - st['m']) * st['r'])
        return [p0, p1, p2]

    def ln_x(b, s):
        def fin(v):
            xn[b * SUB:(b + 1) * SUB, :] = v
            xnb[s] = _u32(v.astype(BF16))
        return ln_passes(lambda: _bf(xbuf[b * (SUB // 2):(b + 1) * (SUB // 2), :]).astype(F32), fin)

    def z2_post(b, s):
        def fin(v):
            z2[b * (SUB // 2):(b + 1) * (SUB // 2), :] = _u32(v[:, 0:FF].astype(BF16))
            z2rt[b] = _u32(jnp.transpose(v[:, FF:FH]).astype(BF16))
        return ln_passes(lambda: ztmp[s], fin)

    def z2_tiles(b, s):
        def tile(j):
            lo = (FH + j * 128) // 2
            t = _gelu(_dot_nt(_bf(xnb[s]), _bf(wint[lo:lo + 64, :])))
            ztmp[s, :, j * 128:(j + 1) * 128] = t
            return t[0:8]

        def rem():
            wr = jnp.concatenate([wint[FF // 2:FH // 2, :], wint[(FH + FF) // 2:FH, :]], axis=0)
            zr = _dot_nt(_bf(wr), _bf(xnb[s]))
            z1rt[b] = zr[0:FR]
            ztmp[s, :, FF:FH] = jnp.transpose(_gelu(zr[FR:2 * FR]))
            return zr[0:8]
        return ([functools.partial(tile, j) for j in range(4)] + [rem]
                + [functools.partial(tile, j) for j in range(4, NFT)])

    def z1_tiles(b, s):
        r0 = pl.multiple_of(b * SUB, SUB)

        def tile(j):
            t = _dot_nt(_bf(xnb[s]), _bf(wint[j * 64:(j + 1) * 64, :]))
            z1[pl.ds(r0, SUB), j * 128:(j + 1) * 128] = t
            return t[0:8]
        return [functools.partial(tile, j) for j in range(NFT)]

    def weave(tiles, *passes):
        for n, t in enumerate(tiles):
            t()
            if n % 2 == 0 and n // 2 < 3:
                for p in passes:
                    p[n // 2]()

    def relayout(J, dst, j0):
        for r in range(0, D // 2, 80):
            ev = wraw[J, pl.ds(2 * r, 80, stride=2), :]
            od = wraw[J, pl.ds(2 * r + 1, 80, stride=2), :]
            dst[2 * (J - j0), r:r + 80, :] = (ev & jnp.uint32(0xFFFF)) | (od << 16)
            dst[2 * (J - j0) + 1, r:r + 80, :] = (ev >> 16) | (od & jnp.uint32(0xFFFF0000))

    def wslab(n):
        return wa[n] if n < NA else wb[n - NA]

    cp_x[0].wait()
    for p in ln_x(0, 0) + ln_x(1, 1):
        p()
    cp_win[0].wait()
    t0, t1 = z2_tiles(0, 0), z2_tiles(1, 1)
    weave(t0[0:4] + t1[0:4])
    start_all(batches[1])
    cp_x[1].wait()
    cp_win[1].wait()
    cp_win[2].wait()
    weave(t0[4:] + t1[4:], ln_x(2, 2), ln_x(3, 3))
    weave(z2_tiles(2, 2), z2_post(0, 0))
    weave(z2_tiles(3, 3), z2_post(1, 1))
    cp_win[3].wait()
    cp_x[2].wait()
    weave(z1_tiles(0, 0), z2_post(2, 2))
    weave(z1_tiles(1, 1), z2_post(3, 3))
    weave(z1_tiles(2, 2), ln_x(4, 0))
    weave(z1_tiles(3, 3))

    def ln_chunked(ld, fin, zero, width):
        n = SUB // NCH
        st = {}

        def mean_of(c, tok):
            m = st['m'][c]
            if tok is None:
                return m
            t = jnp.concatenate([_bits(tok) & zero] * (n // 8), axis=0)
            mb = pltpu.bitcast(_bits(jnp.broadcast_to(m, (n, 128))) | t, F32)
            return jnp.concatenate([mb] * (-(-width // 128)), axis=1)[:, 0:width]

        def run(stage, c, tok):
            if stage == 0:
                st['m'] = [jnp.mean(ld(q * n, n), axis=-1, keepdims=True) for q in range(NCH)]
                st['r'] = [None] * NCH
            elif stage == 1:
                m = mean_of(c, tok)
                d = ld(c * n, n) - m
                st['r'][c] = lax.rsqrt(jnp.mean(d * d, axis=-1, keepdims=True) + EPS)
            else:
                m = mean_of(c, tok)
                fin(c * n, n, (ld(c * n, n) - m) * st['r'][c])
        return run

    def ph1(i, carry):
        b0 = 4 + i * P1B
        ch = (b0 + 2) // 2

        @pl.when(ch < 8)
        def _():
            wait_rows(xbuf, ch * 256, 256, SEM_X + ch)
        wait_wgroup(i, i * JP1, JP1)
        zero = lax.shift_right_logical(i, 8)
        for u in range(P1B):
            b = b0 + u
            bn = jnp.minimum(b + 1, NBLK - 1)
            sn = (u + 1) % P1B
            vrem = {}

            def ldx(r, n, bn=bn):
                return _bf(xbuf[pl.ds(pl.multiple_of(bn * (SUB // 2) + r // 2, 8), n // 2), :]).astype(F32)

            def finx(r, n, v, bn=bn, sn=sn):
                xn[pl.ds(pl.multiple_of(bn * SUB + r, 16), n), :] = v
                xnb[sn, r // 2:(r + n) // 2, :] = _u32(v.astype(BF16))

            def ldz(r, n, u=u):
                return ztmp[u, r:r + n, :]

            def finz(r, n, v, b=b, vrem=vrem):
                z2[pl.ds(pl.multiple_of(b * (SUB // 2) + r // 2, 8), n // 2), :] = _u32(v[:, 0:FF].astype(BF16))
                vrem[r] = v[:, FF:FH]
                if r + n == SUB:
                    vr = jnp.concatenate([vrem[k] for k in sorted(vrem)], axis=0)
                    z2rt[b] = _u32(jnp.transpose(vr).astype(BF16))
            lns = {'x': ln_chunked(ldx, finx, zero, D), 'z': ln_chunked(ldz, finz, zero, FH)}
            for n, t in enumerate(z2_tiles(b, u) + z1_tiles(b, u)):
                tok = t()
                for which, stage, c, anchored in LN_PLAN.get(n, []):
                    lns[which](stage, c, tok if anchored else None)
        for jj in range(JP1):
            relayout(i * JP1 + jj, wa, 0)
        return carry
    lax.fori_loop(0, N1, ph1, 0)

    cp_wout.wait()

    def g_unit(g0, nrows, j):
        gh = pl.multiple_of(g0 // 2, 8)
        g = _dot(_bf(wsp[pl.ds(gh, nrows // 2), :]), _bf(z2[:, j * 128:(j + 1) * 128]))
        g = g + bcol[pl.ds(g0, nrows), :]
        u = (_gelu(z1[pl.ds(g0, nrows), j * 128:(j + 1) * 128]) * g).astype(BF16)
        ubuf[0:nrows // 2, j * 128:(j + 1) * 128] = _u32(u)

    def r_unit(b):
        h0 = pl.multiple_of(b * (SUB // 2), SUB // 2)
        lhs = jnp.concatenate([z2rt[k] for k in range(NBLK)], axis=1)
        gt = _dot_nt(_bf(lhs), _bf(wsp[pl.ds(h0, SUB // 2), :]))
        ut = _gelu(z1rt[b]) * (gt + brow[pl.ds(b, 1), :])
        urem[pl.ds(h0, SUB // 2), :] = _u32(jnp.transpose(ut).astype(BF16))

    def m_unit(g0, nrows, c):
        gh = pl.multiple_of(g0 // 2, 8)
        u = jnp.concatenate([ubuf[0:nrows // 2, :], urem[pl.ds(gh, nrows // 2), :]], axis=1)
        gm = _dot(_bf(u), _bf(wout[:, c * 128:(c + 1) * 128]))
        gate[pl.ds(g0, nrows), c * 128:(c + 1) * 128] = gm * jax.nn.sigmoid(gm)

    def ph2(m, carry):
        wait_rows(wsp, m * WSPR, WSPR, SEM_WSP + m)
        j0 = N1 * JP1 + m * JP2
        wait_wgroup(N1 + m, j0, JP2)
        nr = P2B * SUB
        g0 = pl.multiple_of(m * nr, nr)
        rb = [m * 2 * P2B + u for u in range(2 * P2B)]
        hq0 = [m * (H // N2) + u for u in range(H // N2)]

        def q0_unit():
            if hq0:
                h = hq0.pop(0)
                qs[h] = _dot(xn[0:16, :].astype(BF16), _bf(wa[h]))[0:8]
        for j in range(NFT):
            g_unit(g0, nr, j)
            q0_unit()
            if j < len(rb):
                r_unit(rb[j])
        for cc in range(5):
            q0_unit()
            m_unit(g0, nr, cc)
        assert not hq0 and len(rb) <= NFT
        for jj in range(JP2):
            relayout(j0 + jj, wb, NA // 2)
        return carry
    lax.fori_loop(0, N2, ph2, 0)
    cp_wo.wait()
    cp_mem0.wait()
    g_unit(R0, GR, 0)

    def pair(i, mem, sched, g0, g0n):
        zero = lax.shift_right_logical(i, 8)
        ok = _mask()
        r0 = pl.multiple_of(i * 64, 64)

        def run_step(hq, hh, first):
            o_ref = oa if first else ob
            sk_pv = SKA_PV if first else SKB_PV
            st, sm, vp, qv = {}, {}, {}, {}
            acc = [None, 0]

            def wo_chunk(h1):
                h0 = acc[1]
                part = _dot(o_ref[:, h0 * 128:h1 * 128].astype(BF16), _bf(wo[h0 * 64:h1 * 64, :]))
                acc[0] = part if acc[0] is None else acc[0] + part
                acc[1] = h1

            def fillers(slot):
                for u in sched.get(('A' if first else 'B') + str(slot), '').split():
                    if u[0] == 'g':
                        g_unit(g0, GR, int(u[1]))
                    elif u[0] == 'n':
                        g_unit(g0n, GR, int(u[1]))
                    elif u[0] == 'm':
                        m_unit(g0, GR, int(u[1]))
                    else:
                        wo_chunk(acc[1] + 4)

            def scores(h):
                q, k, _ = st[h]
                s = jnp.where(ok, _dot_nt(q, k) * qscale, -1e9 * LOG2E)
                sm[h] = dict(s=s, mx=jnp.max(s, axis=-1, keepdims=True))

            def exps(h):
                d = sm[h]
                d['e'] = jnp.exp2(d['s'] - d['mx'])
                d['l'] = jnp.sum(d['e'], axis=-1, keepdims=True)

            base = 8 if first else 24
            shifts = list(range(-7, 9))

            def vpu_scores(h):
                q8 = (qs[h] if first else qv.pop(h)) * qscale
                row = lax.broadcasted_iota(I32, (8, 1), 0)
                ss = []
                for d in shifts:
                    sj = jnp.sum(q8 * kvf[h, pl.ds(2 * (base + d), 8, stride=2), :], axis=-1, keepdims=True)
                    if d < 0:
                        sj = jnp.where(row >= -d, sj, -jnp.inf)
                    ss.append(sj)
                vp[h] = dict(ss=ss, mx=_tree(jnp.maximum, ss))

            def vpu_out(h):
                dd = vp[h]
                es = [jnp.exp2(sj - dd['mx']) for sj in dd['ss']]
                l = _tree(jnp.add, es)
                o = _tree(jnp.add, [e * kvf[h, pl.ds(2 * (base + d) + 1, 8, stride=2), :]
                                    for e, d in zip(es, shifts)])
                o = o * _recip(l)
                dd['o'] = o
                ro = 32 if first else 40
                ob[ro:ro + 8, h * 128:(h + 1) * 128] = o

            def put_kv(h, pos, rows):
                kvf[h, pl.ds(2 * pos, 8, stride=2), :] = rows[:, 0:128]
                kvf[h, pl.ds(2 * pos + 1, 8, stride=2), :] = rows[:, 128:256]

            def normalize(h):
                d = sm.pop(h)
                p = d['e'] * _recip(d['l'])
                toks32, toks8 = [], []
                if h + 2 < H:
                    toks32.append(sm[h + 2]['s'] - sm[h + 2]['mx'])
                if 0 <= h + 2 - VLAG < H:
                    toks8.append(jnp.broadcast_to(vp[h + 2 - VLAG]['mx'], (8, 40)))
                if h + 1 < H:
                    toks32.append(jnp.broadcast_to(sm[h + 1]['l'], (32, 40)))
                if 0 <= h + 1 - VLAG < H:
                    toks8.append(vp[h + 1 - VLAG]['o'][:, 0:40])
                if toks32 and not first:
                    p = pltpu.bitcast((_tree(jnp.bitwise_or, [_bits(x) for x in toks32]) & zero) | _bits(p), F32)
                if toks8:
                    p0 = pltpu.bitcast((_tree(jnp.bitwise_or, [_bits(x) for x in toks8]) & zero)
                                       | _bits(p[0:8]), F32)
                    p = jnp.concatenate([p0, p[8:32]], axis=0)
                st[h] = (p.astype(BF16), st[h][2])

            def pv(h):
                p, v = st.pop(h)
                o_ref[0:32, h * 128:(h + 1) * 128] = _dot(p, v)

            assert SK_S + 1 + VLAG <= sk_pv + 1
            for t in range(H + sk_pv + 1):
                if t < H:
                    h = t
                    qf = _dot(hq, _bf(wslab(h)))
                    q = qf[0:32].astype(BF16)
                    kv = _dot(hh, _bf(jnp.concatenate([wslab(H + h), wslab(2 * H + h)], axis=1)))
                    if first:
                        put_kv(h, 8, kv[0:8])
                        put_kv(h, 16, kv[32:40])
                        put_kv(h, 32, kv[40:48])
                        k = kv[0:40, 0:128].astype(BF16)
                        v = kv[0:40, 128:256].astype(BF16)
                    else:
                        qv[h] = qf[32:40]
                        qs[h] = qf[40:48]
                        put_kv(h, 24, kv[0:8])
                        k = jnp.concatenate([kv[:, 0:128], kvf[h, pl.ds(64, 8, stride=2), :]], axis=0).astype(BF16)
                        v = jnp.concatenate([kv[:, 128:256], kvf[h, pl.ds(65, 8, stride=2), :]], axis=0).astype(BF16)
                    st[h] = (q, k, v)
                fillers(t)
                for lag, stage in ((sk_pv, pv), (SK_S, scores), (SK_S + VLAG, vpu_scores), (SK_S + 1, exps),
                                   (SK_S + 1 + VLAG, vpu_out), (SK_S + 2, normalize)):
                    if 0 <= t - lag < H:
                        stage(t - lag)
            wo_chunk(H)
            res = acc[0]
            fillers('end')
            return res

        xt = xn[pl.ds(r0, 64), :]
        ha = jnp.concatenate([mem, xt[8:32], xt[0:8], xt[32:40]], axis=0).astype(BF16)
        sa = run_step(ha[0:32], ha, True)
        mem = sa[0:8]
        hb = jnp.concatenate([mem, xt[40:64]], axis=0).astype(BF16)
        rn = pl.multiple_of(jnp.minimum(r0 + 64, S - 8), 8)
        hx = jnp.concatenate([xt[32:40], xn[pl.ds(rn, 8), :]], axis=0).astype(BF16)
        sb = run_step(jnp.concatenate([hb, hx], axis=0), hb, False)
        mem = sb[0:8]
        sall = jnp.concatenate([sb[32:40], sa[8:32], sb[40:48], sb[8:32]], axis=0)
        xr = _bf(xbuf[pl.ds(pl.multiple_of(i * 32, 32), 32), :]).astype(F32)
        obuf[pl.ds(r0, 64), :] = (xr + sall * gate[pl.ds(r0, 64), :]).astype(BF16)
        return mem

    def body(ii, mem):
        g0 = pl.multiple_of(R0 + ii * GR, 16)
        g0n = pl.multiple_of(R0 + jnp.minimum(ii + 1, NBODY - 1) * GR, 16)
        for u in range(UNR):
            mem = pair(ii * UNR + u, mem, SCHED[u], g0, g0n)
        r0 = pl.multiple_of(ii * (64 * UNR), 64 * UNR)
        pltpu.make_async_copy(obuf.at[pl.ds(r0, 64 * UNR), :], out_hbm.at[pl.ds(r0, 64 * UNR), :], osem).start()
        return mem

    lax.fori_loop(0, NBODY, body, mem0_ref[...].astype(F32))
    pltpu.make_async_copy(obuf, out_hbm, osem).wait()


@functools.partial(jax.jit, static_argnames=("A_seg_len",))
def pallas_recurrent_scan__memory_aug_recurrent_mem_tr__mixer_gmlp__prompt_kernel(A_x, A_mem0, A_Wq, A_Wk, A_Wv, A_Wo, A_seg_len, B_x, B_w_in, B_w_sp, B_b_sp, B_w_out):
    assert A_seg_len == SEG and A_x.shape == (1, S, D) and A_mem0.shape == (1, M, D)
    any_spec = pl.BlockSpec(memory_space=pl.ANY)
    out = pl.pallas_call(
        _kernel,
        out_shape=jax.ShapeDtypeStruct((S, D), BF16),
        in_specs=[any_spec] * 10,
        out_specs=any_spec,
        scratch_shapes=[
            pltpu.VMEM((S // 2, D), U32),
            pltpu.VMEM((S, D), F32),
            pltpu.VMEM((4, SUB // 2, D), U32),
            pltpu.VMEM((NJ, D + 8, DH), U32),
            pltpu.VMEM((NA, D // 2, DH), U32),
            pltpu.VMEM((3 * H - NA, D // 2, DH), U32),
            pltpu.VMEM((H * DH // 2, D), U32),
            pltpu.VMEM((FH, D), U32),
            pltpu.VMEM((S // 2, S), U32),
            pltpu.VMEM((FH // 2, D), U32),
            pltpu.VMEM((S, FF), F32),
            pltpu.VMEM((NBLK, FR, SUB), F32),
            pltpu.VMEM((S // 2, FF), U32),
            pltpu.VMEM((NBLK, FR // 2, SUB), U32),
            pltpu.VMEM((4, SUB, FH), F32),
            pltpu.VMEM((S, 128), F32),
            pltpu.VMEM((16, 128), F32),
            pltpu.VMEM((S, D), F32),
            pltpu.VMEM((P2B * SUB // 2, FF), U32),
            pltpu.VMEM((S // 2, FR), U32),
            pltpu.VMEM((H, 88, DH), F32),
            pltpu.VMEM((H, 8, DH), F32),
            pltpu.VMEM((32, H * DH), F32),
            pltpu.VMEM((48, H * DH), F32),
            pltpu.VMEM((S, D), BF16),
            pltpu.VMEM((M, D), BF16),
            pltpu.VMEM((16, 128), BF16),
            pltpu.SemaphoreType.DMA((NSEM,)),
            pltpu.SemaphoreType.DMA,
        ],
        compiler_params=pltpu.CompilerParams(vmem_limit_bytes=110 * 1024 * 1024),
    )(A_x.reshape(S, D), A_mem0.reshape(M, D), A_Wq, A_Wk, A_Wv, A_Wo.reshape(H * DH, D),
      B_w_in.T, B_w_sp, B_b_sp.reshape(16, 128), B_w_out)
    return out.reshape(1, S, D)
```

```python
import functools

import jax
import jax.numpy as jnp
from jax import lax
import jax.experimental.pallas as pl
import jax.experimental.pallas.tpu as pltpu

F32 = jnp.float32
BF16 = jnp.bfloat16
U32 = jnp.uint32
I32 = jnp.int32

S, D, H, DH, M, SEG = 2048, 640, 32, 128, 8, 32
FH = 864
FF = 768
FR = FH - FF
NFT = FF // 128
EPS = 1e-5
LOG2E = 1.4426950408889634

NPAIR = S // (2 * SEG)
UNR = 2
NBODY = NPAIR // UNR
SUB = 128
NBLK = S // SUB
R0 = 1024
GR = (S - R0) // NBODY
P1B = 2
P2B = 2
N1 = (NBLK - 4) // P1B
N2 = (R0 // SUB) // P2B
NJ = 3 * H // 2
JP1 = 4
JP2 = (NJ - N1 * JP1) // N2
NA = 2 * N1 * JP1
WSPR = S // N2
assert N1 * JP1 + N2 * JP2 == NJ and NA >= H

SK_S, SKA_PV, SKB_PV, VLAG = 2, 5, 7, 3
SCHED = (
    {'A32': 'g1', 'A33': 'w', 'A34': 'w', 'A35': 'w', 'A36': 'w', 'Aend': 'g2',
     'B32': 'g3', 'B33': 'w', 'B34': 'w', 'B35': 'w', 'B36': 'w', 'Bend': 'g4'},
    {'A32': 'g5', 'A33': 'w', 'A34': 'w', 'A35': 'w', 'A36': 'w', 'Aend': 'm0 m1',
     'B32': 'm2 m3', 'B33': 'm4', 'B34': 'w', 'B35': 'w', 'B36': 'w', 'Bend': 'n0'},
)
NCH = 4
LN_PLAN = {
    0: [('x', 0, 0, 0)], 1: [('x', 1, 0, 1)], 2: [('x', 1, 1, 1)], 3: [('x', 1, 2, 1), ('x', 1, 3, 1)],
    4: [('x', 2, 0, 1)], 6: [('z', 0, 0, 0)],
    7: [('z', 1, 0, 0), ('z', 1, 1, 0), ('z', 1, 2, 0), ('z', 1, 3, 0)],
    8: [('z', 2, 0, 0), ('z', 2, 1, 0)], 9: [('z', 2, 2, 1), ('x', 2, 1, 1)],
    10: [('z', 2, 3, 1), ('x', 2, 2, 1)], 11: [('x', 2, 3, 1)],
}

SEM_X = 0
SEM_WIN = 8
SEM_W = 11
SEM_WOUT = SEM_W + N1 + N2
SEM_WSP = SEM_WOUT + 1
SEM_WO = SEM_WSP + N2
SEM_SMALL = SEM_WO + 1
NSEM = SEM_SMALL + 2


def _bf(x):
    return pltpu.bitcast(x, BF16)


def _u32(x):
    return pltpu.bitcast(x, U32)


def _bits(x):
    return pltpu.bitcast(x, I32)


def _dot(a, b):
    return jnp.dot(a, b, preferred_element_type=F32)


def _dot_nt(a, b):
    return lax.dot_general(a, b, (((1,), (1,)), ((), ())), preferred_element_type=F32)


def _gelu(x):
    c = 0.7978845608028654
    t = jnp.tanh(x * (c + (c * 0.044715) * (x * x)))
    hx = 0.5 * x
    return hx + hx * t


def _recip(l):
    r = pl.reciprocal(l, approx=True)
    return r * (2.0 - l * r)


def _tree(op, xs):
    xs = list(xs)
    while len(xs) > 1:
        xs = [op(xs[n], xs[n + 1]) if n + 1 < len(xs) else xs[n] for n in range(0, len(xs), 2)]
    return xs[0]


def _mask():
    qi = lax.broadcasted_iota(I32, (32, 40), 0)
    ki = lax.broadcasted_iota(I32, (32, 40), 1)
    return (qi < 8) | (ki < 8) | (ki >= 32) | (qi >= ki)


def _kernel(x_hbm, mem0_hbm, wq_hbm, wk_hbm, wv_hbm, wo_hbm, wint_hbm, wsp_hbm, bsp_hbm, wout_hbm,
            out_hbm,
            xbuf, xn, xnb, wraw, wa, wb, wo, wint, wsp, wout, z1, z1rt, z2, z2rt, ztmp, bcol, brow,
            gate, ubuf, urem, kvf, qs, oa, ob, obuf, mem0_ref, bsp_ref, sems, osem):
    qscale = DH ** -0.5 * LOG2E

    w32 = [w.bitcast(U32) for w in (wq_hbm, wk_hbm, wv_hbm)]
    x32 = x_hbm.bitcast(U32)
    wsp32 = wsp_hbm.bitcast(U32)
    wint32 = wint_hbm.bitcast(U32)

    def cp_rows(src, dst, r0, n, sem):
        return pltpu.make_async_copy(src.at[pl.ds(r0 // 2, n // 2)], dst.at[pl.ds(r0 // 2, n // 2)], sems.at[sem])

    def wait_rows(dst, r0, n, sem):
        d = dst.at[pl.ds(pl.multiple_of(r0 // 2, 8), n // 2)]
        pltpu.make_async_copy(d, d, sems.at[sem]).wait()

    def wgroup(k):
        j0, n = (k * JP1, JP1) if k < N1 else (N1 * JP1 + (k - N1) * JP2, JP2)
        return [pltpu.make_async_copy(w32[J // 16].at[:, J % 16, :], wraw.at[J, pl.ds(0, D)], sems.at[SEM_W + k])
                for J in range(j0, j0 + n)]

    def wait_wgroup(k, j0, n):
        wgrp = wraw.at[pl.ds(j0, n), pl.ds(0, D)]
        pltpu.make_async_copy(wgrp, wgrp, sems.at[SEM_W + k]).wait()

    cp_x = [cp_rows(x32, xbuf, j * 256, 256, SEM_X + j) for j in range(8)]
    cp_win = [cp_rows(wint32, wint, FH, 512, SEM_WIN), cp_rows(wint32, wint, FH + 512, FH - 512, SEM_WIN + 1),
              cp_rows(wint32, wint, FF, FR, SEM_WIN + 1), cp_rows(wint32, wint, 0, FF, SEM_WIN + 2)]
    cp_wout = pltpu.make_async_copy(wout_hbm.bitcast(U32), wout, sems.at[SEM_WOUT])
    cp_wsp = [cp_rows(wsp32, wsp, m * WSPR, WSPR, SEM_WSP + m) for m in range(N2)]
    cp_wo = pltpu.make_async_copy(wo_hbm.bitcast(U32), wo, sems.at[SEM_WO])
    cp_bsp = pltpu.make_async_copy(bsp_hbm, bsp_ref, sems.at[SEM_SMALL])
    cp_mem0 = pltpu.make_async_copy(mem0_hbm, mem0_ref, sems.at[SEM_SMALL + 1])

    dma = [cp_bsp, cp_x[0], cp_win[0], cp_x[1], cp_mem0, cp_win[1], cp_win[2], cp_win[3], cp_x[2]]
    for k in range(N1):
        dma += cp_x[3 + k:4 + k] + wgroup(k)
    dma += [cp_wout]
    for m in range(N2):
        dma += [cp_wsp[m]] + wgroup(N1 + m)
        if m == N2 - 2:
            dma.append(cp_wo)
    batches = [dma[0:50], dma[50:]]

    def start_all(cps):
        for c in cps:
            c.start()

    start_all(batches[0])

    cp_bsp.wait()
    bsp = bsp_ref[...].astype(F32)
    brow[...] = bsp
    kvf[:, 0:16, :] = jnp.zeros((H, 16, DH), F32)
    for c in range(16):
        bcol[c * 128:(c + 1) * 128, :] = jnp.transpose(jnp.broadcast_to(bsp[c:c + 1, :], (128, 128)))

    def ln_passes(ld, fin):
        st = {}

        def p0():
            st['m'] = jnp.mean(ld(), axis=-1, keepdims=True)

        def p1():
            c = ld() - st['m']
            st['r'] = lax.rsqrt(jnp.mean(c * c, axis=-1, keepdims=True) + EPS)

        def p2():
            fin((ld() - st['m']) * st['r'])
        return [p0, p1, p2]

    def ln_x(b, s):
        def fin(v):
            xn[b * SUB:(b + 1) * SUB, :] = v
            xnb[s] = _u32(v.astype(BF16))
        return ln_passes(lambda: _bf(xbuf[b * (SUB // 2):(b + 1) * (SUB // 2), :]).astype(F32), fin)

    def z2_post(b, s):
        def fin(v):
            z2[b * (SUB // 2):(b + 1) * (SUB // 2), :] = _u32(v[:, 0:FF].astype(BF16))
            z2rt[b] = _u32(jnp.transpose(v[:, FF:FH]).astype(BF16))
        return ln_passes(lambda: ztmp[s], fin)

    def z2_tiles(b, s):
        def tile(j):
            lo = (FH + j * 128) // 2
            t = _gelu(_dot_nt(_bf(xnb[s]), _bf(wint[lo:lo + 64, :])))
            ztmp[s, :, j * 128:(j + 1) * 128] = t
            return t[0:8]

        def rem():
            wr = jnp.concatenate([wint[FF // 2:FH // 2, :], wint[(FH + FF) // 2:FH, :]], axis=0)
            zr = _dot_nt(_bf(wr), _bf(xnb[s]))
            z1rt[b] = zr[0:FR]
            ztmp[s, :, FF:FH] = jnp.transpose(_gelu(zr[FR:2 * FR]))
            return zr[0:8]
        return ([functools.partial(tile, j) for j in range(4)] + [rem]
                + [functools.partial(tile, j) for j in range(4, NFT)])

    def z1_tiles(b, s):
        r0 = pl.multiple_of(b * SUB, SUB)

        def tile(j):
            t = _dot_nt(_bf(xnb[s]), _bf(wint[j * 64:(j + 1) * 64, :]))
            z1[pl.ds(r0, SUB), j * 128:(j + 1) * 128] = t
            return t[0:8]
        return [functools.partial(tile, j) for j in range(NFT)]

    def weave(tiles, *passes):
        for n, t in enumerate(tiles):
            t()
            if n % 2 == 0 and n // 2 < 3:
                for p in passes:
                    p[n // 2]()

    def relayout(J, dst, j0):
        for r in range(0, D // 2, 80):
            ev = wraw[J, pl.ds(2 * r, 80, stride=2), :]
            od = wraw[J, pl.ds(2 * r + 1, 80, stride=2), :]
            dst[2 * (J - j0), r:r + 80, :] = (ev & jnp.uint32(0xFFFF)) | (od << 16)
            dst[2 * (J - j0) + 1, r:r + 80, :] = (ev >> 16) | (od & jnp.uint32(0xFFFF0000))

    def wslab(n):
        return wa[n] if n < NA else wb[n - NA]

    cp_x[0].wait()
    for p in ln_x(0, 0) + ln_x(1, 1):
        p()
    cp_win[0].wait()
    t0, t1 = z2_tiles(0, 0), z2_tiles(1, 1)
    weave(t0[0:4] + t1[0:4])
    start_all(batches[1])
    cp_x[1].wait()
    cp_win[1].wait()
    cp_win[2].wait()
    weave(t0[4:] + t1[4:], ln_x(2, 2), ln_x(3, 3))
    weave(z2_tiles(2, 2), z2_post(0, 0))
    weave(z2_tiles(3, 3), z2_post(1, 1))
    cp_win[3].wait()
    cp_x[2].wait()
    weave(z1_tiles(0, 0), z2_post(2, 2))
    weave(z1_tiles(1, 1), z2_post(3, 3))
    weave(z1_tiles(2, 2), ln_x(4, 0))
    weave(z1_tiles(3, 3))

    def ln_chunked(ld, fin, zero, width):
        n = SUB // NCH
        st = {}

        def mean_of(c, tok):
            m = st['m'][c]
            if tok is None:
                return m
            t = jnp.concatenate([_bits(tok) & zero] * (n // 8), axis=0)
            mb = pltpu.bitcast(_bits(jnp.broadcast_to(m, (n, 128))) | t, F32)
            return jnp.concatenate([mb] * (-(-width // 128)), axis=1)[:, 0:width]

        def run(stage, c, tok):
            if stage == 0:
                st['m'] = [jnp.mean(ld(q * n, n), axis=-1, keepdims=True) for q in range(NCH)]
                st['r'] = [None] * NCH
            elif stage == 1:
                m = mean_of(c, tok)
                d = ld(c * n, n) - m
                st['r'][c] = lax.rsqrt(jnp.mean(d * d, axis=-1, keepdims=True) + EPS)
            else:
                m = mean_of(c, tok)
                fin(c * n, n, (ld(c * n, n) - m) * st['r'][c])
        return run

    def ph1(i, carry):
        b0 = 4 + i * P1B
        ch = (b0 + 2) // 2

        @pl.when(ch < 8)
        def _():
            wait_rows(xbuf, ch * 256, 256, SEM_X + ch)
        wait_wgroup(i, i * JP1, JP1)
        zero = lax.shift_right_logical(i, 8)
        for u in range(P1B):
            b = b0 + u
            bn = jnp.minimum(b + 1, NBLK - 1)
            sn = (u + 1) % P1B
            vrem = {}

            def ldx(r, n, bn=bn):
                return _bf(xbuf[pl.ds(pl.multiple_of(bn * (SUB // 2) + r // 2, 8), n // 2), :]).astype(F32)

            def finx(r, n, v, bn=bn, sn=sn):
                xn[pl.ds(pl.multiple_of(bn * SUB + r, 16), n), :] = v
                xnb[sn, r // 2:(r + n) // 2, :] = _u32(v.astype(BF16))

            def ldz(r, n, u=u):
                return ztmp[u, r:r + n, :]

            def finz(r, n, v, b=b, vrem=vrem):
                z2[pl.ds(pl.multiple_of(b * (SUB // 2) + r // 2, 8), n // 2), :] = _u32(v[:, 0:FF].astype(BF16))
                vrem[r] = v[:, FF:FH]
                if r + n == SUB:
                    vr = jnp.concatenate([vrem[k] for k in sorted(vrem)], axis=0)
                    z2rt[b] = _u32(jnp.transpose(vr).astype(BF16))
            lns = {'x': ln_chunked(ldx, finx, zero, D), 'z': ln_chunked(ldz, finz, zero, FH)}
            for n, t in enumerate(z2_tiles(b, u) + z1_tiles(b, u)):
                tok = t()
                for which, stage, c, anchored in LN_PLAN.get(n, []):
                    lns[which](stage, c, tok if anchored else None)
        for jj in range(JP1):
            relayout(i * JP1 + jj, wa, 0)
        return carry
    lax.fori_loop(0, N1, ph1, 0)

    cp_wout.wait()

    def g_unit(g0, nrows, j):
        gh = pl.multiple_of(g0 // 2, 8)
        g = _dot(_bf(wsp[pl.ds(gh, nrows // 2), :]), _bf(z2[:, j * 128:(j + 1) * 128]))
        g = g + bcol[pl.ds(g0, nrows), :]
        u = (_gelu(z1[pl.ds(g0, nrows), j * 128:(j + 1) * 128]) * g).astype(BF16)
        ubuf[0:nrows // 2, j * 128:(j + 1) * 128] = _u32(u)

    def r_unit(b):
        h0 = pl.multiple_of(b * (SUB // 2), SUB // 2)
        lhs = jnp.concatenate([z2rt[k] for k in range(NBLK)], axis=1)
        gt = _dot_nt(_bf(lhs), _bf(wsp[pl.ds(h0, SUB // 2), :]))
        ut = _gelu(z1rt[b]) * (gt + brow[pl.ds(b, 1), :])
        urem[pl.ds(h0, SUB // 2), :] = _u32(jnp.transpose(ut).astype(BF16))

    def m_unit(g0, nrows, c):
        gh = pl.multiple_of(g0 // 2, 8)
        u = jnp.concatenate([ubuf[0:nrows // 2, :], urem[pl.ds(gh, nrows // 2), :]], axis=1)
        gm = _dot(_bf(u), _bf(wout[:, c * 128:(c + 1) * 128]))
        hg = 0.5 * gm
        gate[pl.ds(g0, nrows), c * 128:(c + 1) * 128] = hg + hg * jnp.tanh(hg)

    def ph2(m, carry):
        wait_rows(wsp, m * WSPR, WSPR, SEM_WSP + m)
        j0 = N1 * JP1 + m * JP2
        wait_wgroup(N1 + m, j0, JP2)
        nr = P2B * SUB
        g0 = pl.multiple_of(m * nr, nr)
        rb = [m * 2 * P2B + u for u in range(2 * P2B)]
        hq0 = [m * (H // N2) + u for u in range(H // N2)]

        def q0_unit():
            if hq0:
                h = hq0.pop(0)
                qs[h] = _dot(xn[0:16, :].astype(BF16), _bf(wa[h]))[0:8]
        for j in range(NFT):
            g_unit(g0, nr, j)
            q0_unit()
            if j < len(rb):
                r_unit(rb[j])
        for cc in range(5):
            q0_unit()
            m_unit(g0, nr, cc)
        assert not hq0 and len(rb) <= NFT
        for jj in range(JP2):
            relayout(j0 + jj, wb, NA // 2)
        return carry
    lax.fori_loop(0, N2, ph2, 0)
    cp_wo.wait()
    cp_mem0.wait()
    g_unit(R0, GR, 0)

    def pair(i, mem, sched, g0, g0n):
        zero = lax.shift_right_logical(i, 8)
        ok = _mask()
        r0 = pl.multiple_of(i * 64, 64)

        def run_step(hq, hh, first):
            o_ref = oa if first else ob
            sk_pv = SKA_PV if first else SKB_PV
            st, sm, vp, qv = {}, {}, {}, {}
            acc = [None, 0]

            def wo_chunk(h1):
                h0 = acc[1]
                part = _dot(o_ref[:, h0 * 128:h1 * 128].astype(BF16), _bf(wo[h0 * 64:h1 * 64, :]))
                acc[0] = part if acc[0] is None else acc[0] + part
                acc[1] = h1

            def fillers(slot):
                for u in sched.get(('A' if first else 'B') + str(slot), '').split():
                    if u[0] == 'g':
                        g_unit(g0, GR, int(u[1]))
                    elif u[0] == 'n':
                        g_unit(g0n, GR, int(u[1]))
                    elif u[0] == 'm':
                        m_unit(g0, GR, int(u[1]))
                    else:
                        wo_chunk(acc[1] + 4)

            def scores(h):
                q, k, _ = st[h]
                s = jnp.where(ok, _dot_nt(q, k) * qscale, -1e9 * LOG2E)
                sm[h] = dict(s=s, mx=jnp.max(s, axis=-1, keepdims=True))

            def exps(h):
                d = sm[h]
                d['e'] = jnp.exp2(d['s'] - d['mx'])
                d['l'] = jnp.sum(d['e'], axis=-1, keepdims=True)

            base = 8 if first else 24
            shifts = list(range(-7, 9))

            def vpu_scores(h):
                q8 = (qs[h] if first else qv.pop(h)) * qscale
                row = lax.broadcasted_iota(I32, (8, 1), 0)
                ss = []
                for d in shifts:
                    sj = jnp.sum(q8 * kvf[h, pl.ds(2 * (base + d), 8, stride=2), :], axis=-1, keepdims=True)
                    if d < 0:
                        sj = jnp.where(row >= -d, sj, -jnp.inf)
                    ss.append(sj)
                vp[h] = dict(ss=ss, mx=_tree(jnp.maximum, ss))

            def vpu_out(h):
                dd = vp[h]
                mx = dd['mx']
                ls, parts = [], []
                for g in range(0, 16, 8):
                    es = [jnp.exp2(sj - mx) for sj in dd['ss'][g:g + 8]]
                    ls.append(_tree(jnp.add, es))
                    parts.append(_tree(jnp.add, [e * kvf[h, pl.ds(2 * (base + d) + 1, 8, stride=2), :]
                                                 for e, d in zip(es, shifts[g:g + 8])]))
                    if g == 0:
                        mx = pltpu.bitcast(_bits(mx) | (_bits(ls[0]) & zero), F32)
                l = _tree(jnp.add, ls)
                o = _tree(jnp.add, parts)
                o = o * _recip(l)
                dd['o'] = o
                ro = 32 if first else 40
                ob[ro:ro + 8, h * 128:(h + 1) * 128] = o

            def put_kv(h, pos, rows):
                kvf[h, pl.ds(2 * pos, 8, stride=2), :] = rows[:, 0:128]
                kvf[h, pl.ds(2 * pos + 1, 8, stride=2), :] = rows[:, 128:256]

            def normalize(h):
                d = sm.pop(h)
                p = d['e'] * _recip(d['l'])
                toks32, toks8 = [], []
                if h + 2 < H:
                    toks32.append(sm[h + 2]['s'] - sm[h + 2]['mx'])
                if 0 <= h + 2 - VLAG < H:
                    toks8.append(jnp.broadcast_to(vp[h + 2 - VLAG]['mx'], (8, 40)))
                if h + 1 < H:
                    toks32.append(jnp.broadcast_to(sm[h + 1]['l'], (32, 40)))
                if 0 <= h + 1 - VLAG < H:
                    toks8.append(vp[h + 1 - VLAG]['o'][:, 0:40])
                if toks32 and not first:
                    p = pltpu.bitcast((_tree(jnp.bitwise_or, [_bits(x) for x in toks32]) & zero) | _bits(p), F32)
                if toks8:
                    p0 = pltpu.bitcast((_tree(jnp.bitwise_or, [_bits(x) for x in toks8]) & zero)
                                       | _bits(p[0:8]), F32)
                    p = jnp.concatenate([p0, p[8:32]], axis=0)
                st[h] = (p.astype(BF16), st[h][2])

            def pv(h):
                p, v = st.pop(h)
                o_ref[0:32, h * 128:(h + 1) * 128] = _dot(p, v)

            assert SK_S + 1 + VLAG <= sk_pv + 1
            for t in range(H + sk_pv + 1):
                if t < H:
                    h = t
                    qf = _dot(hq, _bf(wslab(h)))
                    q = qf[0:32].astype(BF16)
                    kv = _dot(hh, _bf(jnp.concatenate([wslab(H + h), wslab(2 * H + h)], axis=1)))
                    if first:
                        put_kv(h, 8, kv[0:8])
                        put_kv(h, 16, kv[32:40])
                        put_kv(h, 32, kv[40:48])
                        k = kv[0:40, 0:128].astype(BF16)
                        v = kv[0:40, 128:256].astype(BF16)
                    else:
                        qv[h] = qf[32:40]
                        qs[h] = qf[40:48]
                        put_kv(h, 24, kv[0:8])
                        k = jnp.concatenate([kv[:, 0:128], kvf[h, pl.ds(64, 8, stride=2), :]], axis=0).astype(BF16)
                        v = jnp.concatenate([kv[:, 128:256], kvf[h, pl.ds(65, 8, stride=2), :]], axis=0).astype(BF16)
                    st[h] = (q, k, v)
                fillers(t)
                for lag, stage in ((sk_pv, pv), (SK_S, scores), (SK_S + VLAG, vpu_scores), (SK_S + 1, exps),
                                   (SK_S + 1 + VLAG, vpu_out), (SK_S + 2, normalize)):
                    if 0 <= t - lag < H:
                        stage(t - lag)
            wo_chunk(H)
            res = acc[0]
            fillers('end')
            return res

        xt = xn[pl.ds(r0, 64), :]
        ha = jnp.concatenate([mem, xt[8:32], xt[0:8], xt[32:40]], axis=0).astype(BF16)
        sa = run_step(ha[0:32], ha, True)
        mem = sa[0:8]
        hb = jnp.concatenate([mem, xt[40:64]], axis=0).astype(BF16)
        rn = pl.multiple_of(jnp.minimum(r0 + 64, S - 8), 8)
        hx = jnp.concatenate([xt[32:40], xn[pl.ds(rn, 8), :]], axis=0).astype(BF16)
        sb = run_step(jnp.concatenate([hb, hx], axis=0), hb, False)
        mem = sb[0:8]
        sall = jnp.concatenate([sb[32:40], sa[8:32], sb[40:48], sb[8:32]], axis=0)
        xr = _bf(xbuf[pl.ds(pl.multiple_of(i * 32, 32), 32), :]).astype(F32)
        obuf[pl.ds(r0, 64), :] = (xr + sall * gate[pl.ds(r0, 64), :]).astype(BF16)
        return mem

    def body(ii, mem):
        g0 = pl.multiple_of(R0 + ii * GR, 16)
        g0n = pl.multiple_of(R0 + jnp.minimum(ii + 1, NBODY - 1) * GR, 16)
        for u in range(UNR):
            mem = pair(ii * UNR + u, mem, SCHED[u], g0, g0n)
        r0 = pl.multiple_of(ii * (64 * UNR), 64 * UNR)
        pltpu.make_async_copy(obuf.at[pl.ds(r0, 64 * UNR), :], out_hbm.at[pl.ds(r0, 64 * UNR), :], osem).start()
        return mem

    lax.fori_loop(0, NBODY, body, mem0_ref[...].astype(F32))
    pltpu.make_async_copy(obuf, out_hbm, osem).wait()


@functools.partial(jax.jit, static_argnames=("A_seg_len",))
def pallas_recurrent_scan__memory_aug_recurrent_mem_tr__mixer_gmlp__prompt_kernel(A_x, A_mem0, A_Wq, A_Wk, A_Wv, A_Wo, A_seg_len, B_x, B_w_in, B_w_sp, B_b_sp, B_w_out):
    assert A_seg_len == SEG and A_x.shape == (1, S, D) and A_mem0.shape == (1, M, D)
    any_spec = pl.BlockSpec(memory_space=pl.ANY)
    out = pl.pallas_call(
        _kernel,
        out_shape=jax.ShapeDtypeStruct((S, D), BF16),
        in_specs=[any_spec] * 10,
        out_specs=any_spec,
        scratch_shapes=[
            pltpu.VMEM((S // 2, D), U32),
            pltpu.VMEM((S, D), F32),
            pltpu.VMEM((4, SUB // 2, D), U32),
            pltpu.VMEM((NJ, D + 8, DH), U32),
            pltpu.VMEM((NA, D // 2, DH), U32),
            pltpu.VMEM((3 * H - NA, D // 2, DH), U32),
            pltpu.VMEM((H * DH // 2, D), U32),
            pltpu.VMEM((FH, D), U32),
            pltpu.VMEM((S // 2, S), U32),
            pltpu.VMEM((FH // 2, D), U32),
            pltpu.VMEM((S, FF), F32),
            pltpu.VMEM((NBLK, FR, SUB), F32),
            pltpu.VMEM((S // 2, FF), U32),
            pltpu.VMEM((NBLK, FR // 2, SUB), U32),
            pltpu.VMEM((4, SUB, FH), F32),
            pltpu.VMEM((S, 128), F32),
            pltpu.VMEM((16, 128), F32),
            pltpu.VMEM((S, D), F32),
            pltpu.VMEM((P2B * SUB // 2, FF), U32),
            pltpu.VMEM((S // 2, FR), U32),
            pltpu.VMEM((H, 88, DH), F32),
            pltpu.VMEM((H, 8, DH), F32),
            pltpu.VMEM((32, H * DH), F32),
            pltpu.VMEM((48, H * DH), F32),
            pltpu.VMEM((S, D), BF16),
            pltpu.VMEM((M, D), BF16),
            pltpu.VMEM((16, 128), BF16),
            pltpu.SemaphoreType.DMA((NSEM,)),
            pltpu.SemaphoreType.DMA,
        ],
        compiler_params=pltpu.CompilerParams(vmem_limit_bytes=110 * 1024 * 1024),
    )(A_x.reshape(S, D), A_mem0.reshape(M, D), A_Wq, A_Wk, A_Wv, A_Wo.reshape(H * DH, D),
      B_w_in.T, B_w_sp, B_b_sp.reshape(16, 128), B_w_out)
    return out.reshape(1, S, D)
```

```python
import functools

import jax
import jax.numpy as jnp
from jax import lax
import jax.experimental.pallas as pl
import jax.experimental.pallas.tpu as pltpu

F32 = jnp.float32
BF16 = jnp.bfloat16
U32 = jnp.uint32
I32 = jnp.int32

S, D, H, DH, M, SEG = 2048, 640, 32, 128, 8, 32
FH = 864
FF = 768
FR = FH - FF
NFT = FF // 128
EPS = 1e-5
LOG2E = 1.4426950408889634

NPAIR = S // (2 * SEG)
UNR = 2
NBODY = NPAIR // UNR
SUB = 128
NBLK = S // SUB
R0 = 1024
GR = (S - R0) // NBODY
P1B = 2
P2B = 2
N1 = (NBLK - 4) // P1B
N2 = (R0 // SUB) // P2B
NJ = 3 * H // 2
JP1 = 4
JP2 = (NJ - N1 * JP1) // N2
NA = 2 * N1 * JP1
WSPR = S // N2
assert N1 * JP1 + N2 * JP2 == NJ and NA >= H

SK_S, SKA_PV, SKB_PV, VLAG = 2, 5, 7, 3
SCHED = (
    {'A32': 'g1', 'A33': 'w', 'A34': 'w', 'A35': 'w', 'A36': 'w', 'Aend': 'g2',
     'B32': 'g3', 'B33': 'w', 'B34': 'w', 'B35': 'w', 'B36': 'w', 'Bend': 'g4'},
    {'A32': 'g5', 'A33': 'w', 'A34': 'w', 'A35': 'w', 'A36': 'w', 'Aend': 'm0 m1',
     'B32': 'm2 m3', 'B33': 'm4', 'B34': 'w', 'B35': 'w', 'B36': 'w', 'Bend': 'n0'},
)
NCH = 4
LN_PLAN = {
    0: [('x', 0, 0, 0)], 1: [('x', 1, 0, 1)], 2: [('x', 1, 1, 1)], 3: [('x', 1, 2, 1), ('x', 1, 3, 1)],
    4: [('x', 2, 0, 1)], 6: [('z', 0, 0, 0)],
    7: [('z', 1, 0, 0), ('z', 1, 1, 0), ('z', 1, 2, 0), ('z', 1, 3, 0)],
    8: [('z', 2, 0, 0), ('z', 2, 1, 0)], 9: [('z', 2, 2, 1), ('x', 2, 1, 1)],
    10: [('z', 2, 3, 1), ('x', 2, 2, 1)], 11: [('x', 2, 3, 1)],
}

SEM_X = 0
SEM_WIN = 8
SEM_W = 11
SEM_WOUT = SEM_W + N1 + N2
SEM_WSP = SEM_WOUT + 1
SEM_WO = SEM_WSP + N2
SEM_SMALL = SEM_WO + 1
NSEM = SEM_SMALL + 2


def _bf(x):
    return pltpu.bitcast(x, BF16)


def _u32(x):
    return pltpu.bitcast(x, U32)


def _bits(x):
    return pltpu.bitcast(x, I32)


def _dot(a, b):
    return jnp.dot(a, b, preferred_element_type=F32)


def _dot_nt(a, b):
    return lax.dot_general(a, b, (((1,), (1,)), ((), ())), preferred_element_type=F32)


def _gelu(x):
    c = 0.7978845608028654
    t = jnp.tanh(x * (c + (c * 0.044715) * (x * x)))
    hx = 0.5 * x
    return hx + hx * t


def _recip(l):
    r = pl.reciprocal(l, approx=True)
    return r * (2.0 - l * r)


def _tree(op, xs):
    xs = list(xs)
    while len(xs) > 1:
        xs = [op(xs[n], xs[n + 1]) if n + 1 < len(xs) else xs[n] for n in range(0, len(xs), 2)]
    return xs[0]


def _mask():
    qi = lax.broadcasted_iota(I32, (32, 40), 0)
    ki = lax.broadcasted_iota(I32, (32, 40), 1)
    return (qi < 8) | (ki < 8) | (ki >= 32) | (qi >= ki)


def _kernel(x_hbm, mem0_hbm, wq_hbm, wk_hbm, wv_hbm, wo_hbm, wint_hbm, wsp_hbm, bsp_hbm, wout_hbm,
            out_hbm,
            xbuf, xn, xnb, wraw, wa, wb, wo, wint, wsp, wout, z1, z1rt, z2, z2rt, ztmp, bcol, brow,
            gate, ubuf, urem, kvf, qs, oa, ob, obuf, mem0_ref, bsp_ref, sems, osem):
    qscale = DH ** -0.5 * LOG2E

    w32 = [w.bitcast(U32) for w in (wq_hbm, wk_hbm, wv_hbm)]
    x32 = x_hbm.bitcast(U32)
    wsp32 = wsp_hbm.bitcast(U32)
    wint32 = wint_hbm.bitcast(U32)

    def cp_rows(src, dst, r0, n, sem):
        return pltpu.make_async_copy(src.at[pl.ds(r0 // 2, n // 2)], dst.at[pl.ds(r0 // 2, n // 2)], sems.at[sem])

    def wait_rows(dst, r0, n, sem):
        d = dst.at[pl.ds(pl.multiple_of(r0 // 2, 8), n // 2)]
        pltpu.make_async_copy(d, d, sems.at[sem]).wait()

    def wgroup(k):
        j0, n = (k * JP1, JP1) if k < N1 else (N1 * JP1 + (k - N1) * JP2, JP2)
        return [pltpu.make_async_copy(w32[J // 16].at[:, J % 16, :], wraw.at[J, pl.ds(0, D)], sems.at[SEM_W + k])
                for J in range(j0, j0 + n)]

    def wait_wgroup(k, j0, n):
        wgrp = wraw.at[pl.ds(j0, n), pl.ds(0, D)]
        pltpu.make_async_copy(wgrp, wgrp, sems.at[SEM_W + k]).wait()

    cp_x = [cp_rows(x32, xbuf, j * 256, 256, SEM_X + j) for j in range(8)]
    cp_win = [cp_rows(wint32, wint, FH, 512, SEM_WIN), cp_rows(wint32, wint, FH + 512, FH - 512, SEM_WIN + 1),
              cp_rows(wint32, wint, FF, FR, SEM_WIN + 1), cp_rows(wint32, wint, 0, FF, SEM_WIN + 2)]
    cp_wout = pltpu.make_async_copy(wout_hbm.bitcast(U32), wout, sems.at[SEM_WOUT])
    cp_wsp = [cp_rows(wsp32, wsp, m * WSPR, WSPR, SEM_WSP + m) for m in range(N2)]
    cp_wo = pltpu.make_async_copy(wo_hbm.bitcast(U32), wo, sems.at[SEM_WO])
    cp_bsp = pltpu.make_async_copy(bsp_hbm, bsp_ref, sems.at[SEM_SMALL])
    cp_mem0 = pltpu.make_async_copy(mem0_hbm, mem0_ref, sems.at[SEM_SMALL + 1])

    dma = [cp_bsp, cp_x[0], cp_win[0], cp_x[1], cp_mem0, cp_win[1], cp_win[2], cp_win[3], cp_x[2]]
    for k in range(N1):
        dma += cp_x[3 + k:4 + k] + wgroup(k)
    dma += [cp_wout]
    for m in range(N2):
        dma += [cp_wsp[m]] + wgroup(N1 + m)
        if m == N2 - 2:
            dma.append(cp_wo)
    batches = [dma[0:50], dma[50:]]

    def start_all(cps):
        for c in cps:
            c.start()

    start_all(batches[0])

    cp_bsp.wait()
    bsp = bsp_ref[...].astype(F32)
    brow[...] = bsp
    kvf[:, 0:16, :] = jnp.zeros((H, 16, DH), F32)
    for c in range(16):
        bcol[c * 128:(c + 1) * 128, :] = jnp.transpose(jnp.broadcast_to(bsp[c:c + 1, :], (128, 128)))

    def ln_passes(ld, fin):
        st = {}

        def p0():
            st['m'] = jnp.mean(ld(), axis=-1, keepdims=True)

        def p1():
            c = ld() - st['m']
            st['r'] = lax.rsqrt(jnp.mean(c * c, axis=-1, keepdims=True) + EPS)

        def p2():
            fin((ld() - st['m']) * st['r'])
        return [p0, p1, p2]

    def ln_x(b, s):
        def fin(v):
            xn[b * SUB:(b + 1) * SUB, :] = v
            xnb[s] = _u32(v.astype(BF16))
        return ln_passes(lambda: _bf(xbuf[b * (SUB // 2):(b + 1) * (SUB // 2), :]).astype(F32), fin)

    def z2_post(b, s):
        def fin(v):
            z2[b * (SUB // 2):(b + 1) * (SUB // 2), :] = _u32(v[:, 0:FF].astype(BF16))
            z2rt[b] = _u32(jnp.transpose(v[:, FF:FH]).astype(BF16))
        return ln_passes(lambda: ztmp[s], fin)

    def z2_tiles(b, s):
        def tile(j):
            lo = (FH + j * 128) // 2
            t = _gelu(_dot_nt(_bf(xnb[s]), _bf(wint[lo:lo + 64, :])))
            ztmp[s, :, j * 128:(j + 1) * 128] = t
            return t[0:8]

        def rem():
            wr = jnp.concatenate([wint[FF // 2:FH // 2, :], wint[(FH + FF) // 2:FH, :]], axis=0)
            zr = _dot_nt(_bf(wr), _bf(xnb[s]))
            z1rt[b] = zr[0:FR]
            ztmp[s, :, FF:FH] = jnp.transpose(_gelu(zr[FR:2 * FR]))
            return zr[0:8]
        return ([functools.partial(tile, j) for j in range(4)] + [rem]
                + [functools.partial(tile, j) for j in range(4, NFT)])

    def z1_tiles(b, s):
        r0 = pl.multiple_of(b * SUB, SUB)

        def tile(j):
            t = _dot_nt(_bf(xnb[s]), _bf(wint[j * 64:(j + 1) * 64, :]))
            z1[pl.ds(r0, SUB), j * 128:(j + 1) * 128] = t
            return t[0:8]
        return [functools.partial(tile, j) for j in range(NFT)]

    def weave(tiles, *passes):
        for n, t in enumerate(tiles):
            t()
            if n % 2 == 0 and n // 2 < 3:
                for p in passes:
                    p[n // 2]()

    def relayout(J, dst, j0):
        for r in range(0, D // 2, 80):
            ev = wraw[J, pl.ds(2 * r, 80, stride=2), :]
            od = wraw[J, pl.ds(2 * r + 1, 80, stride=2), :]
            dst[2 * (J - j0), r:r + 80, :] = (ev & jnp.uint32(0xFFFF)) | (od << 16)
            dst[2 * (J - j0) + 1, r:r + 80, :] = (ev >> 16) | (od & jnp.uint32(0xFFFF0000))

    def wslab(n):
        return wa[n] if n < NA else wb[n - NA]

    cp_x[0].wait()
    for p in ln_x(0, 0) + ln_x(1, 1):
        p()
    cp_win[0].wait()
    t0, t1 = z2_tiles(0, 0), z2_tiles(1, 1)
    weave(t0[0:4] + t1[0:4])
    start_all(batches[1])
    cp_x[1].wait()
    cp_win[1].wait()
    cp_win[2].wait()
    weave(t0[4:] + t1[4:], ln_x(2, 2), ln_x(3, 3))
    weave(z2_tiles(2, 2), z2_post(0, 0))
    weave(z2_tiles(3, 3), z2_post(1, 1))
    cp_win[3].wait()
    cp_x[2].wait()
    weave(z1_tiles(0, 0), z2_post(2, 2))
    weave(z1_tiles(1, 1), z2_post(3, 3))
    weave(z1_tiles(2, 2), ln_x(4, 0))
    weave(z1_tiles(3, 3))

    def ln_chunked(ld, fin, zero, width):
        n = SUB // NCH
        st = {}

        def mean_of(c, tok):
            m = st['m'][c]
            if tok is None:
                return m
            t = jnp.concatenate([_bits(tok) & zero] * (n // 8), axis=0)
            mb = pltpu.bitcast(_bits(jnp.broadcast_to(m, (n, 128))) | t, F32)
            return jnp.concatenate([mb] * (-(-width // 128)), axis=1)[:, 0:width]

        def run(stage, c, tok):
            if stage == 0:
                st['m'] = [jnp.mean(ld(q * n, n), axis=-1, keepdims=True) for q in range(NCH)]
                st['r'] = [None] * NCH
            elif stage == 1:
                m = mean_of(c, tok)
                d = ld(c * n, n) - m
                st['r'][c] = lax.rsqrt(jnp.mean(d * d, axis=-1, keepdims=True) + EPS)
            else:
                m = mean_of(c, tok)
                fin(c * n, n, (ld(c * n, n) - m) * st['r'][c])
        return run

    def ph1(i, carry):
        b0 = 4 + i * P1B
        ch = (b0 + 2) // 2

        @pl.when(ch < 8)
        def _():
            wait_rows(xbuf, ch * 256, 256, SEM_X + ch)
        wait_wgroup(i, i * JP1, JP1)
        zero = lax.shift_right_logical(i, 8)
        for u in range(P1B):
            b = b0 + u
            bn = jnp.minimum(b + 1, NBLK - 1)
            sn = (u + 1) % P1B
            vrem = {}

            def ldx(r, n, bn=bn):
                return _bf(xbuf[pl.ds(pl.multiple_of(bn * (SUB // 2) + r // 2, 8), n // 2), :]).astype(F32)

            def finx(r, n, v, bn=bn, sn=sn):
                xn[pl.ds(pl.multiple_of(bn * SUB + r, 16), n), :] = v
                xnb[sn, r // 2:(r + n) // 2, :] = _u32(v.astype(BF16))

            def ldz(r, n, u=u):
                return ztmp[u, r:r + n, :]

            def finz(r, n, v, b=b, vrem=vrem):
                z2[pl.ds(pl.multiple_of(b * (SUB // 2) + r // 2, 8), n // 2), :] = _u32(v[:, 0:FF].astype(BF16))
                vrem[r] = v[:, FF:FH]
                if r + n == SUB:
                    vr = jnp.concatenate([vrem[k] for k in sorted(vrem)], axis=0)
                    z2rt[b] = _u32(jnp.transpose(vr).astype(BF16))
            lns = {'x': ln_chunked(ldx, finx, zero, D), 'z': ln_chunked(ldz, finz, zero, FH)}
            for n, t in enumerate(z2_tiles(b, u) + z1_tiles(b, u)):
                tok = t()
                for which, stage, c, anchored in LN_PLAN.get(n, []):
                    lns[which](stage, c, tok if anchored else None)
        for jj in range(JP1):
            relayout(i * JP1 + jj, wa, 0)
        return carry
    lax.fori_loop(0, N1, ph1, 0)

    cp_wout.wait()

    def g_unit(g0, nrows, j):
        gh = pl.multiple_of(g0 // 2, 8)
        g = _dot(_bf(wsp[pl.ds(gh, nrows // 2), :]), _bf(z2[:, j * 128:(j + 1) * 128]))
        g = g + bcol[pl.ds(g0, nrows), :]
        u = (_gelu(z1[pl.ds(g0, nrows), j * 128:(j + 1) * 128]) * g).astype(BF16)
        ubuf[0:nrows // 2, j * 128:(j + 1) * 128] = _u32(u)

    def r_unit(b):
        h0 = pl.multiple_of(b * (SUB // 2), SUB // 2)
        lhs = jnp.concatenate([z2rt[k] for k in range(NBLK)], axis=1)
        gt = _dot_nt(_bf(lhs), _bf(wsp[pl.ds(h0, SUB // 2), :]))
        ut = _gelu(z1rt[b]) * (gt + brow[pl.ds(b, 1), :])
        urem[pl.ds(h0, SUB // 2), :] = _u32(jnp.transpose(ut).astype(BF16))

    def m_unit(g0, nrows, c):
        gh = pl.multiple_of(g0 // 2, 8)
        u = jnp.concatenate([ubuf[0:nrows // 2, :], urem[pl.ds(gh, nrows // 2), :]], axis=1)
        gm = _dot(_bf(u), _bf(wout[:, c * 128:(c + 1) * 128]))
        hg = 0.5 * gm
        gate[pl.ds(g0, nrows), c * 128:(c + 1) * 128] = hg + hg * jnp.tanh(hg)

    def ph2(m, carry):
        wait_rows(wsp, m * WSPR, WSPR, SEM_WSP + m)
        j0 = N1 * JP1 + m * JP2
        wait_wgroup(N1 + m, j0, JP2)
        nr = P2B * SUB
        g0 = pl.multiple_of(m * nr, nr)
        rb = [m * 2 * P2B + u for u in range(2 * P2B)]
        hq0 = [m * (H // N2) + u for u in range(H // N2)]

        def q0_unit():
            if hq0:
                h = hq0.pop(0)
                qs[h] = _dot(xn[0:16, :].astype(BF16), _bf(wa[h]))[0:8]
        for j in range(NFT):
            g_unit(g0, nr, j)
            if j < len(rb):
                r_unit(rb[j])
            q0_unit()
        for cc in range(5):
            q0_unit()
            m_unit(g0, nr, cc)
        assert not hq0 and len(rb) <= NFT
        for jj in range(JP2):
            relayout(j0 + jj, wb, NA // 2)
        return carry
    lax.fori_loop(0, N2, ph2, 0)
    cp_wo.wait()
    cp_mem0.wait()
    g_unit(R0, GR, 0)

    def pair(i, mem, sched, g0, g0n):
        zero = lax.shift_right_logical(i, 8)
        ok = _mask()
        r0 = pl.multiple_of(i * 64, 64)

        def run_step(hq, hh, first):
            o_ref = oa if first else ob
            sk_pv = SKA_PV if first else SKB_PV
            st, sm, vp, qv = {}, {}, {}, {}
            acc = [None, 0]

            def wo_chunk(h1):
                h0 = acc[1]
                part = _dot(o_ref[:, h0 * 128:h1 * 128].astype(BF16), _bf(wo[h0 * 64:h1 * 64, :]))
                acc[0] = part if acc[0] is None else acc[0] + part
                acc[1] = h1

            def fillers(slot):
                for u in sched.get(('A' if first else 'B') + str(slot), '').split():
                    if u[0] == 'g':
                        g_unit(g0, GR, int(u[1]))
                    elif u[0] == 'n':
                        g_unit(g0n, GR, int(u[1]))
                    elif u[0] == 'm':
                        m_unit(g0, GR, int(u[1]))
                    else:
                        wo_chunk(acc[1] + 4)

            def scores(h):
                q, k, _ = st[h]
                s = jnp.where(ok, _dot_nt(q, k) * qscale, -1e9 * LOG2E)
                sm[h] = dict(s=s, mx=jnp.max(s, axis=-1, keepdims=True))

            def exps(h):
                d = sm[h]
                d['e'] = jnp.exp2(d['s'] - d['mx'])
                d['l'] = jnp.sum(d['e'], axis=-1, keepdims=True)

            base = 8 if first else 24
            shifts = list(range(-7, 9))

            def vpu_scores(h):
                q8 = (qs[h] if first else qv.pop(h)) * qscale
                row = lax.broadcasted_iota(I32, (8, 1), 0)
                ss = []
                for d in shifts:
                    sj = jnp.sum(q8 * kvf[h, pl.ds(2 * (base + d), 8, stride=2), :], axis=-1, keepdims=True)
                    if d < 0:
                        sj = jnp.where(row >= -d, sj, -jnp.inf)
                    ss.append(sj)
                vp[h] = dict(ss=ss, mx=_tree(jnp.maximum, ss))

            def vpu_out(h):
                dd = vp[h]
                mx = dd['mx']
                ls, parts = [], []
                for g in range(0, 16, 8):
                    es = [jnp.exp2(sj - mx) for sj in dd['ss'][g:g + 8]]
                    ls.append(_tree(jnp.add, es))
                    parts.append(_tree(jnp.add, [e * kvf[h, pl.ds(2 * (base + d) + 1, 8, stride=2), :]
                                                 for e, d in zip(es, shifts[g:g + 8])]))
                    if g == 0:
                        mx = pltpu.bitcast(_bits(mx) | (_bits(ls[0]) & zero), F32)
                l = _tree(jnp.add, ls)
                o = _tree(jnp.add, parts)
                o = o * _recip(l)
                dd['o'] = o
                ro = 32 if first else 40
                ob[ro:ro + 8, h * 128:(h + 1) * 128] = o

            def put_kv(h, pos, rows):
                kvf[h, pl.ds(2 * pos, 8, stride=2), :] = rows[:, 0:128]
                kvf[h, pl.ds(2 * pos + 1, 8, stride=2), :] = rows[:, 128:256]

            def normalize(h):
                d = sm.pop(h)
                p = d['e'] * _recip(d['l'])
                toks32, toks8 = [], []
                if h + 2 < H:
                    toks32.append(sm[h + 2]['s'] - sm[h + 2]['mx'])
                if 0 <= h + 2 - VLAG < H:
                    toks8.append(jnp.broadcast_to(vp[h + 2 - VLAG]['mx'], (8, 40)))
                if h + 1 < H:
                    toks32.append(jnp.broadcast_to(sm[h + 1]['l'], (32, 40)))
                if 0 <= h + 1 - VLAG < H:
                    toks8.append(vp[h + 1 - VLAG]['o'][:, 0:40])
                if toks32 and not first:
                    p = pltpu.bitcast((_tree(jnp.bitwise_or, [_bits(x) for x in toks32]) & zero) | _bits(p), F32)
                if toks8:
                    p0 = pltpu.bitcast((_tree(jnp.bitwise_or, [_bits(x) for x in toks8]) & zero)
                                       | _bits(p[0:8]), F32)
                    p = jnp.concatenate([p0, p[8:32]], axis=0)
                st[h] = (p.astype(BF16), st[h][2])

            def pv(h):
                p, v = st.pop(h)
                o_ref[0:32, h * 128:(h + 1) * 128] = _dot(p, v)

            assert SK_S + 1 + VLAG <= sk_pv + 1
            for t in range(H + sk_pv + 1):
                if t < H:
                    h = t
                    qf = _dot(hq, _bf(wslab(h)))
                    q = qf[0:32].astype(BF16)
                    kv = _dot(hh, _bf(jnp.concatenate([wslab(H + h), wslab(2 * H + h)], axis=1)))
                    if first:
                        put_kv(h, 8, kv[0:8])
                        put_kv(h, 16, kv[32:40])
                        put_kv(h, 32, kv[40:48])
                        k = kv[0:40, 0:128].astype(BF16)
                        v = kv[0:40, 128:256].astype(BF16)
                    else:
                        qv[h] = qf[32:40]
                        qs[h] = qf[40:48]
                        put_kv(h, 24, kv[0:8])
                        k = jnp.concatenate([kv[:, 0:128], kvf[h, pl.ds(64, 8, stride=2), :]], axis=0).astype(BF16)
                        v = jnp.concatenate([kv[:, 128:256], kvf[h, pl.ds(65, 8, stride=2), :]], axis=0).astype(BF16)
                    st[h] = (q, k, v)
                fillers(t)
                for lag, stage in ((sk_pv, pv), (SK_S, scores), (SK_S + VLAG, vpu_scores), (SK_S + 1, exps),
                                   (SK_S + 1 + VLAG, vpu_out), (SK_S + 2, normalize)):
                    if 0 <= t - lag < H:
                        stage(t - lag)
            wo_chunk(H)
            res = acc[0]
            fillers('end')
            return res

        xt = xn[pl.ds(r0, 64), :]
        ha = jnp.concatenate([mem, xt[8:32], xt[0:8], xt[32:40]], axis=0).astype(BF16)
        sa = run_step(ha[0:32], ha, True)
        mem = sa[0:8]
        hb = jnp.concatenate([mem, xt[40:64]], axis=0).astype(BF16)
        rn = pl.multiple_of(jnp.minimum(r0 + 64, S - 8), 8)
        hx = jnp.concatenate([xt[32:40], xn[pl.ds(rn, 8), :]], axis=0).astype(BF16)
        sb = run_step(jnp.concatenate([hb, hx], axis=0), hb, False)
        mem = sb[0:8]
        sall = jnp.concatenate([sb[32:40], sa[8:32], sb[40:48], sb[8:32]], axis=0)
        xr = _bf(xbuf[pl.ds(pl.multiple_of(i * 32, 32), 32), :]).astype(F32)
        obuf[pl.ds(r0, 64), :] = (xr + sall * gate[pl.ds(r0, 64), :]).astype(BF16)
        return mem

    def body(ii, mem):
        g0 = pl.multiple_of(R0 + ii * GR, 16)
        g0n = pl.multiple_of(R0 + jnp.minimum(ii + 1, NBODY - 1) * GR, 16)
        for u in range(UNR):
            mem = pair(ii * UNR + u, mem, SCHED[u], g0, g0n)
        r0 = pl.multiple_of(ii * (64 * UNR), 64 * UNR)
        pltpu.make_async_copy(obuf.at[pl.ds(r0, 64 * UNR), :], out_hbm.at[pl.ds(r0, 64 * UNR), :], osem).start()
        return mem

    lax.fori_loop(0, NBODY, body, mem0_ref[...].astype(F32))
    pltpu.make_async_copy(obuf, out_hbm, osem).wait()


def _compiler_params():
    vmem = 110 * 1024 * 1024
    try:
        return pltpu.CompilerParams(vmem_limit_bytes=vmem, disable_bounds_checks=True,
                                    disable_semaphore_checks=True)
    except TypeError:
        return pltpu.CompilerParams(vmem_limit_bytes=vmem)


@jax.jit
def pallas_recurrent_scan__memory_aug_recurrent_mem_tr__mixer_gmlp__prompt_kernel(A_x, A_mem0, A_Wq, A_Wk, A_Wv, A_Wo, A_seg_len, B_x, B_w_in, B_w_sp, B_b_sp, B_w_out):
    assert A_x.shape == (1, S, D) and A_mem0.shape == (1, M, D)
    any_spec = pl.BlockSpec(memory_space=pl.ANY)
    out = pl.pallas_call(
        _kernel,
        out_shape=jax.ShapeDtypeStruct((S, D), BF16),
        in_specs=[any_spec] * 10,
        out_specs=any_spec,
        scratch_shapes=[
            pltpu.VMEM((S // 2, D), U32),
            pltpu.VMEM((S, D), F32),
            pltpu.VMEM((4, SUB // 2, D), U32),
            pltpu.VMEM((NJ, D + 8, DH), U32),
            pltpu.VMEM((NA, D // 2, DH), U32),
            pltpu.VMEM((3 * H - NA, D // 2, DH), U32),
            pltpu.VMEM((H * DH // 2, D), U32),
            pltpu.VMEM((FH, D), U32),
            pltpu.VMEM((S // 2, S), U32),
            pltpu.VMEM((FH // 2, D), U32),
            pltpu.VMEM((S, FF), F32),
            pltpu.VMEM((NBLK, FR, SUB), F32),
            pltpu.VMEM((S // 2, FF), U32),
            pltpu.VMEM((NBLK, FR // 2, SUB), U32),
            pltpu.VMEM((4, SUB, FH), F32),
            pltpu.VMEM((S, 128), F32),
            pltpu.VMEM((16, 128), F32),
            pltpu.VMEM((S, D), F32),
            pltpu.VMEM((P2B * SUB // 2, FF), U32),
            pltpu.VMEM((S // 2, FR), U32),
            pltpu.VMEM((H, 88, DH), F32),
            pltpu.VMEM((H, 8, DH), F32),
            pltpu.VMEM((32, H * DH), F32),
            pltpu.VMEM((48, H * DH), F32),
            pltpu.VMEM((S, D), BF16),
            pltpu.VMEM((M, D), BF16),
            pltpu.VMEM((16, 128), BF16),
            pltpu.SemaphoreType.DMA((NSEM,)),
            pltpu.SemaphoreType.DMA,
        ],
        compiler_params=_compiler_params(),
    )(A_x.reshape(S, D), A_mem0.reshape(M, D), A_Wq, A_Wk, A_Wv, A_Wo.reshape(H * DH, D),
      B_w_in.T, B_w_sp, B_b_sp.reshape(16, 128), B_w_out)
    return out.reshape(1, S, D)
```
